```python
import jax
import jax.numpy as jnp

def _softmax(x, axis=-1):
    return jax.nn.softmax(x, axis=axis)
def _gelu(x):
    return jax.nn.gelu(x, approximate=True)
def _silu(x):
    return jax.nn.silu(x)
def _sigmoid(x):
    return jax.nn.sigmoid(x)
def _layernorm(x, axis=-1, eps=1e-5):
    m = jnp.mean(x, axis=axis, keepdims=True)
    v = jnp.var(x, axis=axis, keepdims=True)
    return (x - m) / jnp.sqrt(v + eps)
def _scatter_add(tgt, idx, src, axis=0):
    return tgt.at[idx].add(src)
def _segment_sum(src, seg, n):
    return jax.ops.segment_sum(src, seg, n)
class _Rng:
    def __init__(self, key):
        self._k = key
    def _next(self):
        self._k, sub = jax.random.split(self._k)
        return sub
    def normal(self, shape):
        return jax.random.normal(self._next(), shape, dtype=jnp.bfloat16)
    def randint(self, lo, hi, shape):
        return jax.random.randint(self._next(), shape, lo, hi, dtype=jnp.int32)
    def uniform(self, shape, lo=0.0, hi=1.0):
        return jax.random.uniform(self._next(), shape, jnp.bfloat16, lo, hi)
    def permutation(self, n):
        return jax.random.permutation(self._next(), n)


kernel_name = 'sequential_preLN__mha_block_cached__moe_arch_mod__decode'

def setup_inputs():
    _rng = _Rng(jax.random.key(int.from_bytes(__import__("os").urandom(4), "little")))
    _w = (lambda a: (lambda t: t.astype(jnp.bfloat16) if jnp.issubdtype(t.dtype, jnp.floating) else t)(jnp.asarray(a)))
    def _A_setup():
        B, Sq, D = 4, 1, 640
        H, Sk, Dh = 32, 8192, 192
        return {
            "x": _w((lambda *s: _rng.normal(s) * 0.05)(B, Sq, D)),
            "k_cache": _w((lambda *s: _rng.normal(s) * 0.05)(B, H, Sk, Dh)),
            "v_cache": _w((lambda *s: _rng.normal(s) * 0.05)(B, H, Sk, Dh)),
            "wq": _w((lambda *s: _rng.normal(s) * 0.05)(D, H * Dh) * (D ** -0.5)),
            "wo": _w((lambda *s: _rng.normal(s) * 0.05)(H * Dh, D) * ((H * Dh) ** -0.5)),
        }
    _A_in = _A_setup()

    def _B_setup():
        B, S, D, F, C = 4, 1, 640, 1536, 1
        return {
            "x": _w((lambda *s: _rng.normal(s) * 0.05)(B, S, D)),
            "w_r": _w((lambda *s: _rng.normal(s) * 0.05)(D)),
            "w_gate": _w((lambda *s: _rng.normal(s) * 0.05)(D, F)),
            "w_up": _w((lambda *s: _rng.normal(s) * 0.05)(D, F)),
            "w_down": _w((lambda *s: _rng.normal(s) * 0.05)(F, D)),
        }
    _B_in = _B_setup()

    return {
        "A_x": _A_in["x"],
        "A_k_cache": _A_in["k_cache"],
        "A_v_cache": _A_in["v_cache"],
        "A_wq": _A_in["wq"],
        "A_wo": _A_in["wo"],
        "B_x": _B_in["x"],
        "B_w_r": _B_in["w_r"],
        "B_w_gate": _B_in["w_gate"],
        "B_w_up": _B_in["w_up"],
        "B_w_down": _B_in["w_down"],
    }

def reference(A_x, A_k_cache, A_v_cache, A_wq, A_wo, B_x, B_w_r, B_w_gate, B_w_up, B_w_down):
    def _A_ref(x, k_cache, v_cache, wq, wo):
        B, Sq, D = x.shape
        H, Dh = 32, 192
        q = (lambda x, *d: x.transpose(*d))((x @ wq).reshape(B, Sq, H, Dh), 0, 2, 1, 3)
        scores = jnp.einsum("bhqd,bhkd->bhqk", q, k_cache) * (Dh ** -0.5)
        p = _softmax(scores, axis=-1)
        o = jnp.einsum("bhqk,bhkd->bhqd", p, v_cache)
        return (lambda x, *d: x.transpose(*d))(o, 0, 2, 1, 3).reshape(B, Sq, H * Dh) @ wo

    def _B_ref(x, w_r, w_gate, w_up, w_down):
        B, S, D = x.shape
        C = 1
        r = x @ w_r
        idx = jnp.argsort(-r, axis=-1)[:, :C]
        idx_e = jnp.repeat(idx.reshape(B, C, 1), D, axis=2)
        x_sel = jnp.take_along_axis(x, idx_e, axis=1)
        g = _silu(x_sel @ w_gate)
        u = x_sel @ w_up
        y = (g * u) @ w_down
        r_sel = _sigmoid(jnp.take_along_axis(r, idx, axis=1))
        y = y * r_sel.reshape(B, C, 1)
        b_off = (jnp.arange(B) * S).reshape(B, 1)
        flat_idx = (idx + b_off).reshape(B * C)
        zero = (x * 0.0).reshape(B * S, D)
        upd = _scatter_add(zero, flat_idx, y.reshape(B * C, D), axis=0)
        return x + upd.reshape(B, S, D)

    x = A_x
    h = x + _A_ref(_layernorm(x, axis=-1), A_k_cache, A_v_cache, A_wq, A_wo)
    h2 = h + _B_ref(_layernorm(h, axis=-1), B_w_r, B_w_gate, B_w_up, B_w_down)
    return h2
```

```python
import functools
import jax
import jax.numpy as jnp
from jax import lax
from jax.experimental import pallas as pl
from jax.experimental.pallas import tpu as pltpu

B, D, H, SK, DH, F = 4, 640, 32, 8192, 192, 1536
BH = B * H
EPS = 1e-5
G = 2
RW = G * DH
NG = BH // G
GPB = H // G
CW = 128
NC = SK // CW


def _ln(x):
    m = jnp.mean(x, axis=-1, keepdims=True)
    xc = x - m
    v = jnp.mean(xc * xc, axis=-1, keepdims=True)
    return xc / jnp.sqrt(v + EPS)


def _make_kernel(R1=320, do_dma=True, do_compute=True, WOC=768, U=2, emb=(0,), nobc=True):
    NWO = (H * DH) // WOC
    NWD = 6
    WDC = F // NWD
    P1 = 1

    def kernel(x_hbm, k_hbm, v_hbm, wq_hbm, wo_hbm, wr_hbm, wg_hbm, wu_hbm, wd_hbm, o_ref,
               ring, wq_v, wo_v, wg_v, wu_v, wd_v, x_v, wr_v, q_s, o_s, s_s,
               rsem, wqsem, wosem, wgsem, wdsem, msem):
        def start_p1(src_hbm, g, c):
            r0 = pl.multiple_of(g * RW, RW)
            c0 = pl.multiple_of(c * CW, CW)
            pltpu.make_async_copy(src_hbm.at[pl.ds(r0, R1), pl.ds(c0, CW)], ring.at[c, pl.ds(0, R1)], rsem.at[c]).start(priority=P1)

        def start_p0(src_hbm, g, c):
            r0 = pl.multiple_of(g * RW, RW)
            c0 = pl.multiple_of(c * CW, CW)
            pltpu.make_async_copy(src_hbm.at[pl.ds(r0 + R1, RW - R1), pl.ds(c0, CW)], ring.at[c, pl.ds(R1, RW - R1)], rsem.at[c]).start(priority=0)

        def wait_slot(c):
            pltpu.make_async_copy(k_hbm.at[pl.ds(0, RW), pl.ds(0, CW)], ring.at[c], rsem.at[c]).wait()

        x_cp = pltpu.make_async_copy(x_hbm, x_v, msem.at[0])
        wr_cp = pltpu.make_async_copy(wr_hbm, wr_v, msem.at[1])
        wq_cp = pltpu.make_async_copy(wq_hbm, wq_v, wqsem.at[0])
        wo_cps = [pltpu.make_async_copy(wo_hbm.at[pl.ds(c * WOC, WOC)], wo_v.at[pl.ds(c * WOC, WOC)], wosem.at[c]) for c in range(NWO)]
        wg_cp = pltpu.make_async_copy(wg_hbm, wg_v, wgsem.at[0])
        wu_cp = pltpu.make_async_copy(wu_hbm, wu_v, wgsem.at[1])
        wd_cps = [pltpu.make_async_copy(wd_hbm.at[pl.ds(c * WDC, WDC)], wd_v.at[pl.ds(c * WDC, WDC)], wdsem.at[c]) for c in range(NWD)]

        x_cp.start()
        wq_cp.start(priority=P1)
        wr_cp.start()
        if do_dma:
            def pro(c, _):
                start_p1(k_hbm, 0, c)
                start_p0(k_hbm, 0, c)
                return 0
            lax.fori_loop(0, NC, pro, 0)

        x_cp.wait()
        x4 = x_v[...].astype(jnp.float32)
        xn = _ln(x4)
        xn8 = jnp.concatenate([xn, jnp.zeros((4, D), jnp.float32)], axis=0).astype(jnp.bfloat16)
        wq_cp.wait()
        rowi = lax.broadcasted_iota(jnp.int32, (8, RW), 0)
        lanei = lax.broadcasted_iota(jnp.int32, (8, RW), 1)
        diag = (lanei // DH) == rowi
        for hp in range(GPB):
            qq = jnp.dot(xn8, wq_v[:, hp * RW:(hp + 1) * RW], preferred_element_type=jnp.float32)
            for b in range(B):
                qb = jnp.broadcast_to(qq[b:b + 1], (8, RW))
                q_s[b * GPB + hp] = jnp.where(diag, qb, 0.0).astype(jnp.bfloat16)

        scale = DH ** -0.5

        def tail_starts():
            for c in wo_cps:
                c.start(priority=P1)
            wg_cp.start(priority=P1)
            wu_cp.start(priority=P1)
            for c in wd_cps:
                c.start(priority=P1)

        if do_dma:
            for c in range(U):
                wait_slot(c)

        def phase_body(n, compute, carry, nxt_hbm, nxt_g, refill, last):
            c0 = n * U
            def guarded(cond, fn):
                if cond is True:
                    fn()
                else:
                    pl.when(cond)(fn)
            pending = []
            for u in range(U):
                carry = compute(c0 + u, carry)
                if do_dma:
                    guarded(refill, functools.partial(start_p1, nxt_hbm, nxt_g, c0 + u))
                    pending.append(c0 + u)
                    if u in emb:
                        guarded(refill, functools.partial(start_p0, nxt_hbm, nxt_g, pending.pop(0)))
            if do_dma:
                nemb = len(emb)
                def waits():
                    pend = list(pending)
                    for u in range(U):
                        wait_slot((c0 + U + u) % NC)
                        if u >= nemb:
                            guarded(refill, functools.partial(start_p0, nxt_hbm, nxt_g, pend.pop(0)))
                    assert not pend
                if last is False:
                    waits()
                else:
                    pl.when(jnp.logical_not(jnp.logical_and(last, n == NC // U - 1)))(waits)
            return carry

        def group(g, carry):
            q8 = q_s[g]

            def kcomp(c, m):
                if do_compute:
                    s = jnp.dot(q8, ring[c], preferred_element_type=jnp.float32)
                    s_s[c] = s
                    m = jnp.maximum(m, s)
                return m
            m = lax.fori_loop(0, NC // U, lambda n, m: phase_body(n, kcomp, m, v_hbm, g, True, False),
                              jnp.full((8, CW), -jnp.inf, jnp.float32))
            mx = jnp.max(m, axis=1, keepdims=True)

            def vcomp(c, carry):
                l, o = carry
                if do_compute:
                    p = jnp.exp((s_s[c] - mx) * scale)
                    l = l + p
                    o = o + lax.dot_general(p.astype(jnp.bfloat16), ring[c], (((1,), (1,)), ((), ())),
                                            preferred_element_type=jnp.float32)
                return l, o

            islast = g == NG - 1

            @pl.when(islast)
            def _():
                if do_dma:
                    tail_starts()
            l, o = lax.fori_loop(0, NC // U, lambda n, cr: phase_body(n, vcomp, cr, k_hbm, g + 1, jnp.logical_not(islast), islast),
                                 (jnp.zeros((8, CW), jnp.float32), jnp.zeros((8, RW), jnp.float32)))
            lsum = jnp.sum(l, axis=1, keepdims=True)
            on = jnp.where(diag, o / lsum, 0.0)
            orow = jnp.sum(on, axis=0, keepdims=True)
            b = g // GPB
            hp = g % GPB
            o_s[hp] = jnp.where(rowi == b, jnp.broadcast_to(orow, (8, RW)), o_s[hp])
            return carry

        o_s[...] = jnp.zeros_like(o_s)
        lax.fori_loop(0, NG, group, 0)
        if not do_dma:
            tail_starts()

        ppc = WOC // RW
        attn = jnp.zeros((8, D), jnp.float32)
        for c in range(NWO):
            oc = jnp.concatenate([o_s[c * ppc + j] for j in range(ppc)], axis=1).astype(jnp.bfloat16)
            wo_cps[c].wait()
            attn = attn + jnp.dot(oc, wo_v[c * WOC:(c + 1) * WOC, :], preferred_element_type=jnp.float32)
        x8 = jnp.concatenate([x4, jnp.zeros((4, D), jnp.float32)], axis=0)
        hh = x8 + attn
        hn = _ln(hh)
        wr_cp.wait()
        wr = wr_v[...].astype(jnp.float32).reshape(1, D)
        r = jnp.sum(hn * wr, axis=-1, keepdims=True)
        gate = jax.nn.sigmoid(r)
        hb = hn.astype(jnp.bfloat16)
        wg_cp.wait()
        gg = jnp.dot(hb, wg_v[...], preferred_element_type=jnp.float32)
        wu_cp.wait()
        uu = jnp.dot(hb, wu_v[...], preferred_element_type=jnp.float32)
        a = (gg * jax.nn.sigmoid(gg) * uu).astype(jnp.bfloat16)
        y = jnp.zeros((8, D), jnp.float32)
        for c in range(NWD):
            wd_cps[c].wait()
            y = y + jnp.dot(a[:, c * WDC:(c + 1) * WDC], wd_v[c * WDC:(c + 1) * WDC, :], preferred_element_type=jnp.float32)
        res = hh + hn + y * gate
        o_ref[...] = res[0:4].astype(o_ref.dtype)

    @jax.jit
    def f(A_x, A_k_cache, A_v_cache, A_wq, A_wo, B_x, B_w_r, B_w_gate, B_w_up, B_w_down):
        kt = jnp.swapaxes(A_k_cache, 2, 3).reshape(BH * DH, SK)
        vt = jnp.swapaxes(A_v_cache, 2, 3).reshape(BH * DH, SK)
        x = A_x.reshape(B, D)
        out = pl.pallas_call(
            kernel,
            out_shape=jax.ShapeDtypeStruct((B, D), jnp.bfloat16),
            in_specs=[pl.BlockSpec(memory_space=pl.ANY)] * 9,
            out_specs=pl.BlockSpec(memory_space=pltpu.VMEM),
            scratch_shapes=[
                pltpu.VMEM((NC, RW, CW), jnp.bfloat16),
                pltpu.VMEM((D, H * DH), jnp.bfloat16),
                pltpu.VMEM((H * DH, D), jnp.bfloat16),
                pltpu.VMEM((D, F), jnp.bfloat16),
                pltpu.VMEM((D, F), jnp.bfloat16),
                pltpu.VMEM((F, D), jnp.bfloat16),
                pltpu.VMEM((B, D), jnp.bfloat16),
                pltpu.VMEM((D,), jnp.bfloat16),
                pltpu.VMEM((NG, 8, RW), jnp.bfloat16),
                pltpu.VMEM((GPB, 8, RW), jnp.float32),
                pltpu.VMEM((NC, 8, CW), jnp.float32),
                pltpu.SemaphoreType.DMA((NC,)),
                pltpu.SemaphoreType.DMA((1,)),
                pltpu.SemaphoreType.DMA((NWO,)),
                pltpu.SemaphoreType.DMA((2,)),
                pltpu.SemaphoreType.DMA((NWD,)),
                pltpu.SemaphoreType.DMA((2,)),
            ],
            compiler_params=pltpu.CompilerParams(vmem_limit_bytes=110 * 1024 * 1024, disable_bounds_checks=nobc),
        )(x, kt, vt, A_wq, A_wo, B_w_r, B_w_gate, B_w_up, B_w_down)
        return out.reshape(B, 1, D)

    return f


_impl = _make_kernel()


@jax.jit
def pallas_sequential_preLN__mha_block_cached__moe_arch_mod__decode_kernel(
    A_x, A_k_cache, A_v_cache, A_wq, A_wo, B_x, B_w_r, B_w_gate, B_w_up, B_w_down):
    return _impl(A_x, A_k_cache, A_v_cache, A_wq, A_wo, B_x, B_w_r, B_w_gate, B_w_up, B_w_down)
```

```python
import functools
import jax
import jax.numpy as jnp
from jax import lax
from jax.experimental import pallas as pl
from jax.experimental.pallas import tpu as pltpu

B, D, H, SK, DH, F = 4, 640, 32, 8192, 192, 1536
BH = B * H
EPS = 1e-5
RW = 2 * DH
NPAIR = BH // 2
PPB = H // 2
CW = 128
NC = SK // CW


def _ln(x):
    m = jnp.mean(x, axis=-1, keepdims=True)
    xc = x - m
    v = jnp.mean(xc * xc, axis=-1, keepdims=True)
    return xc / jnp.sqrt(v + EPS)


def _make_kernel(R1=352, NP=2, CPI=1, emb=(0,), do_dma=True, do_compute=True, WOC=768, nobc=False):
    NWO = (H * DH) // WOC
    NWD = 6
    WDC = F // NWD
    P1 = 1
    NSG = NPAIR // NP
    NS = NC * NP
    U = CPI * NP
    NIT = NS // U

    def kernel(x_hbm, k_hbm, v_hbm, wq_hbm, wo_hbm, wr_hbm, wg_hbm, wu_hbm, wd_hbm, o_ref,
               ring, wq_v, wo_v, wg_v, wu_v, wd_v, x_v, wr_v, q_s, o_s, s_s,
               rsem, wqsem, wosem, wgsem, wdsem, msem):
        def src_off(sg, c, j):
            r0 = pl.multiple_of((sg * NP + j) * RW, RW)
            c0 = pl.multiple_of(c * CW, CW)
            return r0, c0

        def start_p1(src_hbm, sg, c, j):
            r0, c0 = src_off(sg, c, j)
            t = c * NP + j
            pltpu.make_async_copy(src_hbm.at[pl.ds(r0, R1), pl.ds(c0, CW)], ring.at[t, pl.ds(0, R1)], rsem.at[t]).start(priority=P1)

        def start_p0(src_hbm, sg, c, j):
            r0, c0 = src_off(sg, c, j)
            t = c * NP + j
            pltpu.make_async_copy(src_hbm.at[pl.ds(r0 + R1, RW - R1), pl.ds(c0, CW)], ring.at[t, pl.ds(R1, RW - R1)], rsem.at[t]).start(priority=0)

        def wait_slot(t):
            pltpu.make_async_copy(k_hbm.at[pl.ds(0, RW), pl.ds(0, CW)], ring.at[t], rsem.at[t]).wait()

        x_cp = pltpu.make_async_copy(x_hbm, x_v, msem.at[0])
        wr_cp = pltpu.make_async_copy(wr_hbm, wr_v, msem.at[1])
        wq_cp = pltpu.make_async_copy(wq_hbm, wq_v, wqsem.at[0])
        wo_cps = [pltpu.make_async_copy(wo_hbm.at[pl.ds(c * WOC, WOC)], wo_v.at[pl.ds(c * WOC, WOC)], wosem.at[c]) for c in range(NWO)]
        wg_cp = pltpu.make_async_copy(wg_hbm, wg_v, wgsem.at[0])
        wu_cp = pltpu.make_async_copy(wu_hbm, wu_v, wgsem.at[1])
        wd_cps = [pltpu.make_async_copy(wd_hbm.at[pl.ds(c * WDC, WDC)], wd_v.at[pl.ds(c * WDC, WDC)], wdsem.at[c]) for c in range(NWD)]

        x_cp.start()
        wq_cp.start(priority=P1)
        wr_cp.start()
        if do_dma:
            def pro(c, _):
                for j in range(NP):
                    start_p1(k_hbm, 0, c, j)
                    start_p0(k_hbm, 0, c, j)
                return 0
            lax.fori_loop(0, NC, pro, 0)

        x_cp.wait()
        x4 = x_v[...].astype(jnp.float32)
        xn = _ln(x4)
        xn8 = jnp.concatenate([xn, jnp.zeros((4, D), jnp.float32)], axis=0).astype(jnp.bfloat16)
        wq_cp.wait()
        rowi = lax.broadcasted_iota(jnp.int32, (8, RW), 0)
        lanei = lax.broadcasted_iota(jnp.int32, (8, RW), 1)
        half = (lanei >= DH).astype(jnp.int32)
        diag = [(rowi == (2 * j + half)) for j in range(NP)]
        for hp in range(PPB):
            qq = jnp.dot(xn8, wq_v[:, hp * RW:(hp + 1) * RW], preferred_element_type=jnp.float32)
            for b in range(B):
                qb = jnp.broadcast_to(qq[b:b + 1], (8, RW))
                q_s[b * PPB + hp] = jnp.where(diag[hp % NP], qb, 0.0).astype(jnp.bfloat16)

        scale = DH ** -0.5

        def tail_starts():
            for c in wo_cps:
                c.start(priority=P1)
            wg_cp.start(priority=P1)
            wu_cp.start(priority=P1)
            for c in wd_cps:
                c.start(priority=P1)

        if do_dma:
            for t in range(U):
                wait_slot(t)

        def guarded(cond, fn):
            if cond is True:
                fn()
            else:
                pl.when(cond)(fn)

        def phase_body(n, pre, compute, post, carry, nxt_hbm, nxt_sg, refill, last):
            pending = []
            u = 0
            for ci in range(CPI):
                c = n * CPI + ci
                carry = pre(c, carry)
                for j in range(NP):
                    carry = compute(c, j, carry)
                    if do_dma:
                        guarded(refill, functools.partial(start_p1, nxt_hbm, nxt_sg, c, j))
                        pending.append((c, j))
                        if u in emb:
                            guarded(refill, functools.partial(start_p0, nxt_hbm, nxt_sg, *pending.pop(0)))
                    u += 1
                carry = post(c, carry)
            if do_dma:
                nemb = len(emb)

                def waits():
                    pend = list(pending)
                    for u in range(U):
                        wait_slot((n * U + U + u) % NS)
                        if u >= nemb:
                            guarded(refill, functools.partial(start_p0, nxt_hbm, nxt_sg, *pend.pop(0)))
                    assert not pend
                if last is False:
                    waits()
                else:
                    pl.when(jnp.logical_not(jnp.logical_and(last, n == NIT - 1)))(waits)
            return carry

        def group(sg, carry):
            qs = [q_s[sg * NP + j] for j in range(NP)]

            def kpre(c, carry):
                return carry[0], jnp.zeros((8, CW), jnp.float32)

            def kcomp(c, j, carry):
                m, s = carry
                if do_compute:
                    sp = jnp.dot(qs[j], ring[c * NP + j], preferred_element_type=jnp.float32)
                    s = sp if j == 0 else s + sp
                return m, s

            def kpost(c, carry):
                m, s = carry
                if do_compute:
                    s_s[c] = s
                    m = jnp.maximum(m, s)
                return m, s

            def kbody(n, m):
                m, _ = phase_body(n, kpre, kcomp, kpost, (m, None), v_hbm, sg, True, False)
                return m
            m = lax.fori_loop(0, NIT, kbody, jnp.full((8, CW), -jnp.inf, jnp.float32))
            mx = jnp.max(m, axis=1, keepdims=True)

            def vpre(c, carry):
                l, os_, _ = carry
                p = None
                if do_compute:
                    p = jnp.exp((s_s[c] - mx) * scale)
                    l = l + p
                    p = p.astype(jnp.bfloat16)
                return l, os_, p

            def vcomp(c, j, carry):
                l, os_, p = carry
                if do_compute:
                    os_ = list(os_)
                    os_[j] = os_[j] + lax.dot_general(p, ring[c * NP + j], (((1,), (1,)), ((), ())),
                                                      preferred_element_type=jnp.float32)
                    os_ = tuple(os_)
                return l, os_, p

            def vpost(c, carry):
                return carry

            islast = sg == NSG - 1

            @pl.when(islast)
            def _():
                if do_dma:
                    tail_starts()

            def vbody(n, cr):
                l, os_, _ = phase_body(n, vpre, vcomp, vpost, (cr[0], cr[1], None), k_hbm, sg + 1, jnp.logical_not(islast), islast)
                return l, os_
            l, os_ = lax.fori_loop(0, NIT, vbody, (jnp.zeros((8, CW), jnp.float32),
                                                   tuple(jnp.zeros((8, RW), jnp.float32) for _ in range(NP))))
            lsum = jnp.sum(l, axis=1, keepdims=True)
            b = (sg * NP) // PPB
            for j in range(NP):
                on = jnp.where(diag[j], os_[j] / lsum, 0.0)
                orow = jnp.sum(on, axis=0, keepdims=True)
                hp = (sg * NP + j) % PPB
                o_s[hp] = jnp.where(rowi == b, jnp.broadcast_to(orow, (8, RW)), o_s[hp])
            return carry

        o_s[...] = jnp.zeros_like(o_s)
        lax.fori_loop(0, NSG, group, 0)
        if not do_dma:
            tail_starts()

        ppc = WOC // RW
        attn = jnp.zeros((8, D), jnp.float32)
        for c in range(NWO):
            oc = jnp.concatenate([o_s[c * ppc + j] for j in range(ppc)], axis=1).astype(jnp.bfloat16)
            wo_cps[c].wait()
            attn = attn + jnp.dot(oc, wo_v[c * WOC:(c + 1) * WOC, :], preferred_element_type=jnp.float32)
        x8 = jnp.concatenate([x4, jnp.zeros((4, D), jnp.float32)], axis=0)
        hh = x8 + attn
        hn = _ln(hh)
        wr_cp.wait()
        wr = wr_v[...].astype(jnp.float32).reshape(1, D)
        r = jnp.sum(hn * wr, axis=-1, keepdims=True)
        gate = jax.nn.sigmoid(r)
        hb = hn.astype(jnp.bfloat16)
        wg_cp.wait()
        gg = jnp.dot(hb, wg_v[...], preferred_element_type=jnp.float32)
        wu_cp.wait()
        uu = jnp.dot(hb, wu_v[...], preferred_element_type=jnp.float32)
        a = (gg * jax.nn.sigmoid(gg) * uu).astype(jnp.bfloat16)
        y = jnp.zeros((8, D), jnp.float32)
        for c in range(NWD):
            wd_cps[c].wait()
            y = y + jnp.dot(a[:, c * WDC:(c + 1) * WDC], wd_v[c * WDC:(c + 1) * WDC, :], preferred_element_type=jnp.float32)
        res = hh + hn + y * gate
        o_ref[...] = res[0:4].astype(o_ref.dtype)

    @jax.jit
    def f(A_x, A_k_cache, A_v_cache, A_wq, A_wo, B_x, B_w_r, B_w_gate, B_w_up, B_w_down):
        kt = jnp.swapaxes(A_k_cache, 2, 3).reshape(BH * DH, SK)
        vt = jnp.swapaxes(A_v_cache, 2, 3).reshape(BH * DH, SK)
        x = A_x.reshape(B, D)
        out = pl.pallas_call(
            kernel,
            out_shape=jax.ShapeDtypeStruct((B, D), jnp.bfloat16),
            in_specs=[pl.BlockSpec(memory_space=pl.ANY)] * 9,
            out_specs=pl.BlockSpec(memory_space=pltpu.VMEM),
            scratch_shapes=[
                pltpu.VMEM((NS, RW, CW), jnp.bfloat16),
                pltpu.VMEM((D, H * DH), jnp.bfloat16),
                pltpu.VMEM((H * DH, D), jnp.bfloat16),
                pltpu.VMEM((D, F), jnp.bfloat16),
                pltpu.VMEM((D, F), jnp.bfloat16),
                pltpu.VMEM((F, D), jnp.bfloat16),
                pltpu.VMEM((B, D), jnp.bfloat16),
                pltpu.VMEM((D,), jnp.bfloat16),
                pltpu.VMEM((NPAIR, 8, RW), jnp.bfloat16),
                pltpu.VMEM((PPB, 8, RW), jnp.float32),
                pltpu.VMEM((NC, 8, CW), jnp.float32),
                pltpu.SemaphoreType.DMA((NS,)),
                pltpu.SemaphoreType.DMA((1,)),
                pltpu.SemaphoreType.DMA((NWO,)),
                pltpu.SemaphoreType.DMA((2,)),
                pltpu.SemaphoreType.DMA((NWD,)),
                pltpu.SemaphoreType.DMA((2,)),
            ],
            compiler_params=pltpu.CompilerParams(vmem_limit_bytes=110 * 1024 * 1024, disable_bounds_checks=nobc),
        )(x, kt, vt, A_wq, A_wo, B_w_r, B_w_gate, B_w_up, B_w_down)
        return out.reshape(B, 1, D)

    return f


_impl = _make_kernel()


@jax.jit
def pallas_sequential_preLN__mha_block_cached__moe_arch_mod__decode_kernel(
    A_x, A_k_cache, A_v_cache, A_wq, A_wo, B_x, B_w_r, B_w_gate, B_w_up, B_w_down):
    return _impl(A_x, A_k_cache, A_v_cache, A_wq, A_wo, B_x, B_w_r, B_w_gate, B_w_up, B_w_down)
```

```python
import functools
import jax
import jax.numpy as jnp
from jax import lax
from jax.experimental import pallas as pl
from jax.experimental.pallas import tpu as pltpu

B, D, H, SK, DH, F = 4, 640, 32, 8192, 192, 1536
BH = B * H
EPS = 1e-5
RW = 2 * DH
NPAIR = BH // 2
PPB = H // 2
CW = 128
NC = SK // CW
NP = 2
NSG = NPAIR // NP
NS = NC * NP


def _ln(x):
    m = jnp.mean(x, axis=-1, keepdims=True)
    xc = x - m
    v = jnp.mean(xc * xc, axis=-1, keepdims=True)
    return xc / jnp.sqrt(v + EPS)


def _make_kernel(R1=352, DL=8, CPI=2, kdep=-1, vdep=-1, extras=True, do_dma=True, do_compute=True, NWD=6, nobc=True, WOR=16,
                early_wo=True, notail=False, DP=16):
    WDC = F // NWD
    P1 = 1
    NWOP = (H * DH) // WOR
    GR, GC = 40, 256
    NGR, NGC = D // GR, F // GC
    NGP = NGR * NGC
    U = CPI * NP
    NIT = NC // CPI

    def kernel(x_hbm, k_hbm, v_hbm, wq_hbm, wo_hbm, wr_hbm, wg_hbm, wu_hbm, wd_hbm, o_ref,
               ring, wq_v, wo_v, wg_v, wu_v, wd_v, x_v, wr_v, q_s, o_s, s_s, attn_s, oacc,
               rsem, wqsem, wosem, wgsem, wdsem, msem):
        def src_off(sg, c, j):
            r0 = pl.multiple_of((sg * NP + j) * RW, RW)
            c0 = pl.multiple_of(c * CW, CW)
            return r0, c0

        def start_p1(src_hbm, sg, c, j):
            r0, c0 = src_off(sg, c, j)
            t = c * NP + j
            pltpu.make_async_copy(src_hbm.at[pl.ds(r0, R1), pl.ds(c0, CW)], ring.at[t, pl.ds(0, R1)], rsem.at[t]).start(priority=P1)

        def start_p0(src_hbm, sg, c, j):
            r0, c0 = src_off(sg, c, j)
            t = c * NP + j
            pltpu.make_async_copy(src_hbm.at[pl.ds(r0 + R1, RW - R1), pl.ds(c0, CW)], ring.at[t, pl.ds(R1, RW - R1)], rsem.at[t]).start(priority=0)

        def wait_slot(t):
            pltpu.make_async_copy(k_hbm.at[pl.ds(0, RW), pl.ds(0, CW)], ring.at[t], rsem.at[t]).wait()

        x_cp = pltpu.make_async_copy(x_hbm, x_v, msem.at[0])
        wr_cp = pltpu.make_async_copy(wr_hbm, wr_v, msem.at[1])
        wq_cp = pltpu.make_async_copy(wq_hbm, wq_v, wqsem.at[0])
        wo_all = pltpu.make_async_copy(wo_hbm, wo_v, wosem.at[0])
        wg_all = pltpu.make_async_copy(wg_hbm, wg_v, wgsem.at[0])
        wu_all = pltpu.make_async_copy(wu_hbm, wu_v, wgsem.at[1])
        wd_cps = [pltpu.make_async_copy(wd_hbm.at[pl.ds(c * WDC, WDC)], wd_v.at[pl.ds(c * WDC, WDC)], wdsem.at[c]) for c in range(NWD)]

        def start_extra(e):
            @pl.when(e < NWOP)
            def _():
                r = pl.multiple_of(jnp.minimum(e, NWOP - 1) * WOR, WOR)
                pltpu.make_async_copy(wo_hbm.at[pl.ds(r, WOR)], wo_v.at[pl.ds(r, WOR)], wosem.at[0]).start(priority=0)
            for k, (w_hbm, w_v) in enumerate([(wg_hbm, wg_v), (wu_hbm, wu_v)]):
                lo = NWOP + k * 128

                @pl.when(jnp.logical_and(e >= lo, e < lo + NGP))
                def _():
                    i = jnp.clip(e - lo, 0, NGP - 1)
                    cc = pl.multiple_of((i // NGR) * GC, GC)
                    r = pl.multiple_of((i % NGR) * GR, 8)
                    pltpu.make_async_copy(w_hbm.at[pl.ds(r, GR), pl.ds(cc, GC)], w_v.at[pl.ds(r, GR), pl.ds(cc, GC)], wgsem.at[k]).start(priority=0)

        x_cp.start()
        wq_cp.start(priority=P1)
        wr_cp.start()
        if do_dma:
            def pro(c, _):
                for j in range(NP):
                    if DP == NC:
                        start_p1(k_hbm, 0, c, j)
                    else:
                        @pl.when(c < DP)
                        def _():
                            start_p1(k_hbm, 0, c, j)
                    if DL == 0:
                        start_p0(k_hbm, 0, c, j)
                    else:
                        @pl.when(c < DL)
                        def _():
                            start_p0(k_hbm, 0, c, j)
                return 0
            lax.fori_loop(0, NC, pro, 0)

        x_cp.wait()
        x4 = x_v[...].astype(jnp.float32)
        xn = _ln(x4)
        xn8 = jnp.concatenate([xn, jnp.zeros((4, D), jnp.float32)], axis=0).astype(jnp.bfloat16)
        wq_cp.wait()
        rowi = lax.broadcasted_iota(jnp.int32, (8, RW), 0)
        lanei = lax.broadcasted_iota(jnp.int32, (8, RW), 1)
        half = (lanei >= DH).astype(jnp.int32)
        diag = [(rowi == (2 * j + half)) for j in range(NP)]
        for hp in range(PPB):
            qq = jnp.dot(xn8, wq_v[:, hp * RW:(hp + 1) * RW], preferred_element_type=jnp.float32)
            for b in range(B):
                qb = jnp.broadcast_to(qq[b:b + 1], (8, RW))
                q_s[b * PPB + hp] = jnp.where(diag[hp % NP], qb, 0.0).astype(jnp.bfloat16)

        scale = DH ** -0.5

        def tail_starts():
            if not extras:
                wo_all.start(priority=P1)
                wg_all.start(priority=P1)
                wu_all.start(priority=P1)
            for c in wd_cps:
                c.start(priority=P1)

        if do_dma:
            for t in range(U):
                wait_slot(t)

        def guarded(cond, fn):
            if cond is True:
                fn()
            else:
                pl.when(cond)(fn)

        def event(c, j, cur_hbm, cur_sg, nxt_hbm, nxt_sg, refill):
            if DL == 0:
                guarded(refill, functools.partial(start_p0, nxt_hbm, nxt_sg, c, j))
            else:
                cc = c + DL
                pl.when(cc < NC)(lambda: start_p0(cur_hbm, cur_sg, jnp.minimum(cc, NC - 1), j))
                cond = cc >= NC if refill is True else jnp.logical_and(refill, cc >= NC)
                pl.when(cond)(lambda: start_p0(nxt_hbm, nxt_sg, jnp.maximum(cc - NC, 0), j))

        def refill_p1(c, j, cur_hbm, cur_sg, nxt_hbm, nxt_sg, refill):
            if DP == NC:
                guarded(refill, functools.partial(start_p1, nxt_hbm, nxt_sg, c, j))
            else:
                cc = c + DP
                pl.when(cc < NC)(lambda: start_p1(cur_hbm, cur_sg, jnp.minimum(cc, NC - 1), j))
                cond = cc >= NC if refill is True else jnp.logical_and(refill, cc >= NC)
                pl.when(cond)(lambda: start_p1(nxt_hbm, nxt_sg, jnp.maximum(cc - NC, 0), j))

        def phase_body(n, compute, carry, cur_hbm, cur_sg, nxt_hbm, nxt_sg, refill, last, extra_idx):
            slots = [(n * CPI + ci, j) for ci in range(CPI) for j in range(NP)]
            carry, post = compute(n, carry)
            if do_dma:
                event(*slots[0], cur_hbm, cur_sg, nxt_hbm, nxt_sg, refill)
                for (c, j) in slots:
                    refill_p1(c, j, cur_hbm, cur_sg, nxt_hbm, nxt_sg, refill)
            post()
            if do_dma:
                notl = None if last is False else jnp.logical_not(jnp.logical_and(last, n == NIT - 1))
                for u in range(U):
                    w = functools.partial(wait_slot, (n * U + U + u) % NS)
                    if notl is None:
                        w()
                    else:
                        pl.when(notl)(w)
                    if u >= 1:
                        event(*slots[u], cur_hbm, cur_sg, nxt_hbm, nxt_sg, refill)
                        if extra_idx is not None and u == U - 1:
                            start_extra(extra_idx)
                if last is not False and DP < NC:
                    pl.when(jnp.logical_and(last, n == (NC - DP) // CPI - 1))(tail_starts)
            return carry

        def group(sg, carry):
            qs = [q_s[sg * NP + j] for j in range(NP)]

            def kcompute(n, m):
                if not do_compute:
                    return m, (lambda: None)
                sps = []
                for ci in range(CPI):
                    for j in range(NP):
                        c = n * CPI + ci
                        sps.append(jnp.dot(qs[j], ring[c * NP + j], preferred_element_type=jnp.float32))
                for i in range(kdep + 1):
                    s_s[i % NP, n * CPI + i // NP] = sps[i]
                ss = [sps[ci * NP] + sps[ci * NP + 1] for ci in range(CPI)]
                for s in ss:
                    m = jnp.maximum(m, s)

                def post():
                    for i in range(kdep + 1, CPI * NP):
                        s_s[i % NP, n * CPI + i // NP] = sps[i]
                return m, post

            def kbody(n, m):
                return phase_body(n, kcompute, m, k_hbm, sg, v_hbm, sg, True, False,
                                  (sg * NIT + n) if extras else None)
            m = lax.fori_loop(0, NIT, kbody, jnp.full((8, CW), -jnp.inf, jnp.float32))
            mx = jnp.max(m, axis=1, keepdims=True)

            def vcompute(n, carry):
                if not do_compute:
                    return carry, (lambda: None)
                l, os_ = carry
                os_ = list(os_)
                parts = []
                for ci in range(CPI):
                    c = n * CPI + ci
                    p = jnp.exp((s_s[0, c] + s_s[1, c] - mx) * scale)
                    l = l + p
                    p = p.astype(jnp.bfloat16)
                    if vdep == -2 and ci == 0:
                        pdep = p
                    for j in range(NP):
                        d = lax.dot_general(p, ring[c * NP + j], (((1,), (1,)), ((), ())), preferred_element_type=jnp.float32)
                        if ci * NP + j == vdep:
                            oacc[...] = oacc[...] + d
                        else:
                            os_[j] = os_[j] + d
                return (l, tuple(os_)), (lambda: None)

            islast = sg == NSG - 1

            @pl.when(islast)
            def _():
                if do_dma and DP == NC:
                    tail_starts()
                if early_wo and (extras and do_dma):
                    wo_all.wait()
                    oc = jnp.concatenate([o_s[i] for i in range(PPB)], axis=1).astype(jnp.bfloat16)
                    attn_s[...] = jnp.dot(oc, wo_v[...], preferred_element_type=jnp.float32)

            oacc[...] = jnp.zeros_like(oacc)

            def vbody(n, cr):
                return phase_body(n, vcompute, cr, v_hbm, sg, k_hbm, sg + 1, jnp.logical_not(islast), islast, None)
            l, os_ = lax.fori_loop(0, NIT, vbody, (jnp.zeros((8, CW), jnp.float32),
                                                   tuple(jnp.zeros((8, RW), jnp.float32) for _ in range(NP))))
            lsum = jnp.sum(l, axis=1, keepdims=True)
            if vdep >= 0:
                os_ = list(os_)
                os_[vdep % NP] = os_[vdep % NP] + oacc[...]
            b = (sg * NP) // PPB
            for j in range(NP):
                on = jnp.where(diag[j], os_[j] / lsum, 0.0)
                orow = jnp.sum(on, axis=0, keepdims=True)
                hp = (sg * NP + j) % PPB
                o_s[hp] = jnp.where(rowi == b, jnp.broadcast_to(orow, (8, RW)), o_s[hp])
            return carry

        o_s[...] = jnp.zeros_like(o_s)
        lax.fori_loop(0, NSG, group, 0)
        if not do_dma:
            wo_all.start(); wg_all.start(); wu_all.start()
            for c in wd_cps:
                c.start(priority=P1)

        if notail:
            if not (early_wo and extras):
                wo_all.wait()
            wr_cp.wait(); wg_all.wait(); wu_all.wait()
            for c in range(NWD):
                wd_cps[c].wait()
            o_ref[...] = x4.astype(o_ref.dtype)
            return
        if early_wo and (extras and do_dma):
            lastp = [jnp.where(rowi == B - 1, o_s[PPB - NP + j], 0.0) for j in range(NP)]
            oc = jnp.concatenate(lastp, axis=1).astype(jnp.bfloat16)
            attn = attn_s[...] + jnp.dot(oc, wo_v[(PPB - NP) * RW:, :], preferred_element_type=jnp.float32)
        else:
            wo_all.wait()
            oc = jnp.concatenate([o_s[i] for i in range(PPB)], axis=1).astype(jnp.bfloat16)
            attn = jnp.dot(oc, wo_v[...], preferred_element_type=jnp.float32)
        x8 = jnp.concatenate([x4, jnp.zeros((4, D), jnp.float32)], axis=0)
        hh = x8 + attn
        hn = _ln(hh)
        wr_cp.wait()
        wr = wr_v[...].astype(jnp.float32).reshape(1, D)
        r = jnp.sum(hn * wr, axis=-1, keepdims=True)
        gate = jax.nn.sigmoid(r)
        hb = hn.astype(jnp.bfloat16)
        wg_all.wait()
        wu_all.wait()
        gg = jnp.dot(hb, wg_v[...], preferred_element_type=jnp.float32)
        uu = jnp.dot(hb, wu_v[...], preferred_element_type=jnp.float32)
        a = (gg * jax.nn.sigmoid(gg) * uu).astype(jnp.bfloat16)
        y = jnp.zeros((8, D), jnp.float32)
        for c in range(NWD):
            wd_cps[c].wait()
            y = y + jnp.dot(a[:, c * WDC:(c + 1) * WDC], wd_v[c * WDC:(c + 1) * WDC, :], preferred_element_type=jnp.float32)
        res = hh + hn + y * gate
        o_ref[...] = res[0:4].astype(o_ref.dtype)

    @jax.jit
    def f(A_x, A_k_cache, A_v_cache, A_wq, A_wo, B_x, B_w_r, B_w_gate, B_w_up, B_w_down):
        kt = jnp.swapaxes(A_k_cache, 2, 3).reshape(BH * DH, SK)
        vt = jnp.swapaxes(A_v_cache, 2, 3).reshape(BH * DH, SK)
        x = A_x.reshape(B, D)
        out = pl.pallas_call(
            kernel,
            out_shape=jax.ShapeDtypeStruct((B, D), jnp.bfloat16),
            in_specs=[pl.BlockSpec(memory_space=pl.ANY)] * 9,
            out_specs=pl.BlockSpec(memory_space=pltpu.VMEM),
            scratch_shapes=[
                pltpu.VMEM((NS, RW, CW), jnp.bfloat16),
                pltpu.VMEM((D, H * DH), jnp.bfloat16),
                pltpu.VMEM((H * DH, D), jnp.bfloat16),
                pltpu.VMEM((D, F), jnp.bfloat16),
                pltpu.VMEM((D, F), jnp.bfloat16),
                pltpu.VMEM((F, D), jnp.bfloat16),
                pltpu.VMEM((B, D), jnp.bfloat16),
                pltpu.VMEM((D,), jnp.bfloat16),
                pltpu.VMEM((NPAIR, 8, RW), jnp.bfloat16),
                pltpu.VMEM((PPB, 8, RW), jnp.float32),
                pltpu.VMEM((NP, NC, 8, CW), jnp.float32),
                pltpu.VMEM((8, D), jnp.float32),
                pltpu.VMEM((8, RW), jnp.float32),
                pltpu.SemaphoreType.DMA((NS,)),
                pltpu.SemaphoreType.DMA((1,)),
                pltpu.SemaphoreType.DMA((1,)),
                pltpu.SemaphoreType.DMA((2,)),
                pltpu.SemaphoreType.DMA((NWD,)),
                pltpu.SemaphoreType.DMA((2,)),
            ],
            compiler_params=pltpu.CompilerParams(vmem_limit_bytes=110 * 1024 * 1024, disable_bounds_checks=nobc),
        )(x, kt, vt, A_wq, A_wo, B_w_r, B_w_gate, B_w_up, B_w_down)
        return out.reshape(B, 1, D)

    return f


_impl = _make_kernel()


@jax.jit
def pallas_sequential_preLN__mha_block_cached__moe_arch_mod__decode_kernel(
    A_x, A_k_cache, A_v_cache, A_wq, A_wo, B_x, B_w_r, B_w_gate, B_w_up, B_w_down):
    return _impl(A_x, A_k_cache, A_v_cache, A_wq, A_wo, B_x, B_w_r, B_w_gate, B_w_up, B_w_down)
```

```python
import functools
import jax
import jax.numpy as jnp
from jax import lax
from jax.experimental import pallas as pl
from jax.experimental.pallas import tpu as pltpu

B, D, H, SK, DH, F = 4, 640, 32, 8192, 192, 1536
BH = B * H
EPS = 1e-5
RW = 2 * DH
NPAIR = BH // 2
PPB = H // 2
CW = 128
NC = SK // CW
NP = 2
NSG = NPAIR // NP
NS = NC * NP
QW = NP * RW
NQB = (H * DH) // QW


def _ln(x):
    m = jnp.mean(x, axis=-1, keepdims=True)
    xc = x - m
    v = jnp.mean(xc * xc, axis=-1, keepdims=True)
    return xc / jnp.sqrt(v + EPS)


def _make_kernel(R1=352, DL=8, DP=16, CPI=2, NWD=6, WOR=16, notail=False, do_compute=True, nobc=True, nosc=True):
    WDC = F // NWD
    P1 = 1
    U = CPI * NP
    NIT = NC // CPI
    QR, QC = D * QW // NIT // RW, RW
    assert QR % 8 == 0 and (D // QR) * (QW // QC) == NIT
    NWOP = (H * DH) // WOR
    GR, GC = 40, 256
    NGR = D // GR
    NGP = NGR * (F // GC)
    E0 = (NQB - 1) * NIT
    assert E0 + NWOP + 2 * NGP <= (NSG - 2) * NIT

    def kernel(x_hbm, k_hbm, v_hbm, wq_hbm, wo_hbm, wr_hbm, wg_hbm, wu_hbm, wd_hbm, o_ref,
               ring, wq_v, wo_v, wg_v, wu_v, wd_v, x_v, wr_v, xn_s, q_s, o_s, s_s, attn_s,
               rsem, wqsem, wosem, wgsem, wdsem, msem):
        def slot_copy(src_hbm, sg, c, j, lo, n):
            r0 = pl.multiple_of((sg * NP + j) * RW, RW)
            c0 = pl.multiple_of(c * CW, CW)
            t = c * NP + j
            return pltpu.make_async_copy(src_hbm.at[pl.ds(r0 + lo, n), pl.ds(c0, CW)], ring.at[t, pl.ds(lo, n)], rsem.at[t])

        def start_p1(src_hbm, sg, c, j):
            slot_copy(src_hbm, sg, c, j, 0, R1).start(priority=P1)

        def start_p0(src_hbm, sg, c, j):
            slot_copy(src_hbm, sg, c, j, R1, RW - R1).start(priority=0)

        def wait_slot(t):
            pltpu.make_async_copy(k_hbm.at[pl.ds(0, RW), pl.ds(0, CW)], ring.at[t], rsem.at[t]).wait()

        def wq_block(blk):
            c0 = pl.multiple_of(blk * QW, QW)
            return pltpu.make_async_copy(wq_hbm.at[:, pl.ds(c0, QW)], wq_v.at[blk], wqsem.at[blk])

        x_cp = pltpu.make_async_copy(x_hbm, x_v, msem.at[0])
        wr_cp = pltpu.make_async_copy(wr_hbm, wr_v, msem.at[1])
        wo_all = pltpu.make_async_copy(wo_hbm, wo_v, wosem.at[0])
        wg_all = pltpu.make_async_copy(wg_hbm, wg_v, wgsem.at[0])
        wu_all = pltpu.make_async_copy(wu_hbm, wu_v, wgsem.at[1])
        wd_cps = [pltpu.make_async_copy(wd_hbm.at[pl.ds(c * WDC, WDC)], wd_v.at[pl.ds(c * WDC, WDC)], wdsem.at[c])
                  for c in range(NWD)]

        def start_extra(e):
            @pl.when(e < E0)
            def _():
                ee = jnp.minimum(e, E0 - 1)
                blk = ee // NIT + 1
                i = ee % NIT
                r = pl.multiple_of((i // (QW // QC)) * QR, 8)
                cc = pl.multiple_of((i % (QW // QC)) * QC, QC)
                pltpu.make_async_copy(wq_hbm.at[pl.ds(r, QR), pl.ds(blk * QW + cc, QC)],
                                      wq_v.at[blk, pl.ds(r, QR), pl.ds(cc, QC)], wqsem.at[blk]).start(priority=0)

            @pl.when(jnp.logical_and(e >= E0, e < E0 + NWOP))
            def _():
                r = pl.multiple_of(jnp.clip(e - E0, 0, NWOP - 1) * WOR, WOR)
                pltpu.make_async_copy(wo_hbm.at[pl.ds(r, WOR)], wo_v.at[pl.ds(r, WOR)], wosem.at[0]).start(priority=0)
            for k, (w_hbm, w_v) in enumerate([(wg_hbm, wg_v), (wu_hbm, wu_v)]):
                lo = E0 + NWOP + k * NGP

                @pl.when(jnp.logical_and(e >= lo, e < lo + NGP))
                def _():
                    i = jnp.clip(e - lo, 0, NGP - 1)
                    cc = pl.multiple_of((i // NGR) * GC, GC)
                    r = pl.multiple_of((i % NGR) * GR, 8)
                    pltpu.make_async_copy(w_hbm.at[pl.ds(r, GR), pl.ds(cc, GC)], w_v.at[pl.ds(r, GR), pl.ds(cc, GC)],
                                          wgsem.at[k]).start(priority=0)

        x_cp.start()
        wq_block(0).start()
        for c in range(DP):
            for j in range(NP):
                start_p1(k_hbm, 0, c, j)
        for c in range(DL):
            for j in range(NP):
                start_p0(k_hbm, 0, c, j)
        wr_cp.start()

        o_s[...] = jnp.zeros_like(o_s)
        x_cp.wait()
        x4 = x_v[...].astype(jnp.float32)
        xn_s[...] = jnp.concatenate([_ln(x4), jnp.zeros((4, D), jnp.float32)], axis=0).astype(jnp.bfloat16)
        rowi = lax.broadcasted_iota(jnp.int32, (8, RW), 0)
        lanei = lax.broadcasted_iota(jnp.int32, (8, RW), 1)
        half = (lanei >= DH).astype(jnp.int32)
        diag = [(rowi == (2 * j + half)) for j in range(NP)]
        scale = DH ** -0.5

        def tail_starts():
            for c in wd_cps:
                c.start(priority=P1)

        def guarded(cond, fn):
            if cond is True:
                fn()
            else:
                pl.when(cond)(fn)

        def ahead(start, dist, c, j, cur_hbm, cur_sg, nxt_hbm, nxt_sg, refill):
            cc = c + dist
            pl.when(cc < NC)(lambda: start(cur_hbm, cur_sg, jnp.minimum(cc, NC - 1), j))
            cond = cc >= NC if refill is True else jnp.logical_and(refill, cc >= NC)
            pl.when(cond)(lambda: start(nxt_hbm, nxt_sg, jnp.maximum(cc - NC, 0), j))

        def phase_body(n, compute, carry, cur_hbm, cur_sg, nxt_hbm, nxt_sg, refill, last, extra_idx):
            slots = [(n * CPI + ci, j) for ci in range(CPI) for j in range(NP)]
            ctx = (cur_hbm, cur_sg, nxt_hbm, nxt_sg, refill)
            carry = compute(n, carry)
            ahead(start_p0, DL, *slots[0], *ctx)
            for (c, j) in slots:
                ahead(start_p1, DP, c, j, *ctx)
            notl = None if last is False else jnp.logical_not(jnp.logical_and(last, n == NIT - 1))
            for u in range(U):
                w = functools.partial(wait_slot, (n * U + U + u) % NS)
                if notl is None:
                    w()
                else:
                    pl.when(notl)(w)
                if u >= 1:
                    ahead(start_p0, DL, *slots[u], *ctx)
            if extra_idx is not None:
                start_extra(extra_idx)
            if last is not False:
                pl.when(jnp.logical_and(last, n == (NC - DP) // CPI - 1))(tail_starts)
            return carry

        for t in range(U):
            wait_slot(t)

        def group(sg, carry):
            @pl.when(sg < NQB)
            def _():
                blk = jnp.minimum(sg, NQB - 1)
                wq_block(blk).wait()
                qq = jnp.dot(xn_s[...], wq_v[blk], preferred_element_type=jnp.float32)
                for j in range(NP):
                    for b in range(B):
                        qb = jnp.broadcast_to(qq[b:b + 1, j * RW:(j + 1) * RW], (8, RW))
                        q_s[b * PPB + blk * NP + j] = jnp.where(diag[j], qb, 0.0).astype(jnp.bfloat16)

            qs = [q_s[sg * NP + j] for j in range(NP)]

            def kcompute(n, m):
                if not do_compute:
                    return m
                for ci in range(CPI):
                    c = n * CPI + ci
                    s = None
                    for j in range(NP):
                        sp = jnp.dot(qs[j], ring[c * NP + j], preferred_element_type=jnp.float32)
                        s = sp if s is None else s + sp
                    s_s[c] = s
                    m = jnp.maximum(m, s)
                return m

            def kbody(n, m):
                return phase_body(n, kcompute, m, k_hbm, sg, v_hbm, sg, True, False, sg * NIT + n)
            m = lax.fori_loop(0, NIT, kbody, jnp.full((8, CW), -jnp.inf, jnp.float32))
            mx = jnp.max(m, axis=1, keepdims=True)

            def vcompute(n, carry):
                if not do_compute:
                    return carry
                l, os_ = carry
                os_ = list(os_)
                for ci in range(CPI):
                    c = n * CPI + ci
                    p = jnp.exp((s_s[c] - mx) * scale)
                    l = l + p
                    p = p.astype(jnp.bfloat16)
                    for j in range(NP):
                        os_[j] = os_[j] + lax.dot_general(p, ring[c * NP + j], (((1,), (1,)), ((), ())),
                                                          preferred_element_type=jnp.float32)
                return l, tuple(os_)

            islast = sg == NSG - 1

            @pl.when(islast)
            def _():
                wo_all.wait()
                oc = jnp.concatenate([o_s[i] for i in range(PPB)], axis=1).astype(jnp.bfloat16)
                attn_s[...] = jnp.dot(oc, wo_v[...], preferred_element_type=jnp.float32)

            def vbody(n, cr):
                return phase_body(n, vcompute, cr, v_hbm, sg, k_hbm, sg + 1, jnp.logical_not(islast), islast, None)
            l, os_ = lax.fori_loop(0, NIT, vbody, (jnp.zeros((8, CW), jnp.float32),
                                                   tuple(jnp.zeros((8, RW), jnp.float32) for _ in range(NP))))
            lsum = jnp.sum(l, axis=1, keepdims=True)
            b = (sg * NP) // PPB
            for j in range(NP):
                on = jnp.where(diag[j], os_[j] / lsum, 0.0)
                orow = jnp.sum(on, axis=0, keepdims=True)
                hp = (sg * NP + j) % PPB
                o_s[hp] = jnp.where(rowi == b, jnp.broadcast_to(orow, (8, RW)), o_s[hp])
            return carry

        lax.fori_loop(0, NSG, group, 0)

        x4 = x_v[...].astype(jnp.float32)
        if notail:
            wr_cp.wait(); wg_all.wait(); wu_all.wait()
            for c in range(NWD):
                wd_cps[c].wait()
            o_ref[...] = x4.astype(o_ref.dtype)
            return
        lastp = [jnp.where(rowi == B - 1, o_s[PPB - NP + j], 0.0) for j in range(NP)]
        oc = jnp.concatenate(lastp, axis=1).astype(jnp.bfloat16)
        attn = attn_s[...] + jnp.dot(oc, wo_v[(PPB - NP) * RW:, :], preferred_element_type=jnp.float32)
        x8 = jnp.concatenate([x4, jnp.zeros((4, D), jnp.float32)], axis=0)
        hh = x8 + attn
        hn = _ln(hh)
        wr_cp.wait()
        wr = wr_v[...].astype(jnp.float32).reshape(1, D)
        r = jnp.sum(hn * wr, axis=-1, keepdims=True)
        gate = jax.nn.sigmoid(r)
        hb = hn.astype(jnp.bfloat16)
        wg_all.wait()
        wu_all.wait()
        gg = jnp.dot(hb, wg_v[...], preferred_element_type=jnp.float32)
        uu = jnp.dot(hb, wu_v[...], preferred_element_type=jnp.float32)
        a = (gg * jax.nn.sigmoid(gg) * uu).astype(jnp.bfloat16)
        y = jnp.zeros((8, D), jnp.float32)
        for c in range(NWD):
            wd_cps[c].wait()
            y = y + jnp.dot(a[:, c * WDC:(c + 1) * WDC], wd_v[c * WDC:(c + 1) * WDC, :], preferred_element_type=jnp.float32)
        res = hh + hn + y * gate
        o_ref[...] = res[0:4].astype(o_ref.dtype)

    @jax.jit
    def f(A_x, A_k_cache, A_v_cache, A_wq, A_wo, B_x, B_w_r, B_w_gate, B_w_up, B_w_down):
        kt = jnp.swapaxes(A_k_cache, 2, 3).reshape(BH * DH, SK)
        vt = jnp.swapaxes(A_v_cache, 2, 3).reshape(BH * DH, SK)
        x = A_x.reshape(B, D)
        out = pl.pallas_call(
            kernel,
            out_shape=jax.ShapeDtypeStruct((B, D), jnp.bfloat16),
            in_specs=[pl.BlockSpec(memory_space=pl.ANY)] * 9,
            out_specs=pl.BlockSpec(memory_space=pltpu.VMEM),
            scratch_shapes=[
                pltpu.VMEM((NS, RW, CW), jnp.bfloat16),
                pltpu.VMEM((NQB, D, QW), jnp.bfloat16),
                pltpu.VMEM((H * DH, D), jnp.bfloat16),
                pltpu.VMEM((D, F), jnp.bfloat16),
                pltpu.VMEM((D, F), jnp.bfloat16),
                pltpu.VMEM((F, D), jnp.bfloat16),
                pltpu.VMEM((B, D), jnp.bfloat16),
                pltpu.VMEM((D,), jnp.bfloat16),
                pltpu.VMEM((8, D), jnp.bfloat16),
                pltpu.VMEM((NPAIR, 8, RW), jnp.bfloat16),
                pltpu.VMEM((PPB, 8, RW), jnp.float32),
                pltpu.VMEM((NC, 8, CW), jnp.float32),
                pltpu.VMEM((8, D), jnp.float32),
                pltpu.SemaphoreType.DMA((NS,)),
                pltpu.SemaphoreType.DMA((NQB,)),
                pltpu.SemaphoreType.DMA((1,)),
                pltpu.SemaphoreType.DMA((2,)),
                pltpu.SemaphoreType.DMA((NWD,)),
                pltpu.SemaphoreType.DMA((2,)),
            ],
            compiler_params=pltpu.CompilerParams(vmem_limit_bytes=100 * 1024 * 1024, disable_bounds_checks=nobc, disable_semaphore_checks=nosc),
        )(x, kt, vt, A_wq, A_wo, B_w_r, B_w_gate, B_w_up, B_w_down)
        return out.reshape(B, 1, D)

    return f


_impl = _make_kernel()


@jax.jit
def pallas_sequential_preLN__mha_block_cached__moe_arch_mod__decode_kernel(
    A_x, A_k_cache, A_v_cache, A_wq, A_wo, B_x, B_w_r, B_w_gate, B_w_up, B_w_down):
    return _impl(A_x, A_k_cache, A_v_cache, A_wq, A_wo, B_x, B_w_r, B_w_gate, B_w_up, B_w_down)
```

```python
import functools

import jax
import jax.numpy as jnp
from jax import lax
from jax.experimental import pallas as pl
from jax.experimental.pallas import tpu as pltpu

B, D, H, SK, DH, F = 4, 640, 32, 8192, 192, 1536
BH = B * H
EPS = 1e-5

RW = 2 * DH
CW = 128
NC = SK // CW
NP = 2
NPAIR = BH // 2
PPB = H // 2
NSG = NPAIR // NP
NS = NC * NP
QW = NP * RW
NQB = (H * DH) // QW

R1 = 352
DP = 12
DL = 8
CPI = 2
U = CPI * NP
NIT = NC // CPI
BULK, URGENT = 1, 0

QR, QC = D * QW // NIT // RW, RW
WOR = 16
NWOP = (H * DH) // WOR
GR, GC = 40, 256
NGR = D // GR
NGP = NGR * (F // GC)
E0 = (NQB - 1) * NIT
NWD = 6
WDC = F // NWD
assert QR % 8 == 0 and (D // QR) * (QW // QC) == NIT
assert E0 + NWOP + 2 * NGP <= (NSG - 2) * NIT


def _ln(x):
    m = jnp.mean(x, axis=-1, keepdims=True)
    xc = x - m
    v = jnp.mean(xc * xc, axis=-1, keepdims=True)
    return xc / jnp.sqrt(v + EPS)


def _kernel(x_hbm, k_hbm, v_hbm, wq_hbm, wo_hbm, wr_hbm, wg_hbm, wu_hbm, wd_hbm, o_ref,
            ring, wq_v, wo_v, wg_v, wu_v, wd_v, x_v, wr_v, xn_s, q_s, o_s, s_s, attn_s,
            rsem, wqsem, wosem, wgsem, wdsem, msem):
    def slot_copy(src_hbm, sg, c, j, lo, n):
        r0 = pl.multiple_of((sg * NP + j) * RW, RW)
        c0 = pl.multiple_of(c * CW, CW)
        t = c * NP + j
        return pltpu.make_async_copy(src_hbm.at[pl.ds(r0 + lo, n), pl.ds(c0, CW)],
                                     ring.at[t, pl.ds(lo, n)], rsem.at[t])

    def start_bulk(src_hbm, sg, c, j):
        slot_copy(src_hbm, sg, c, j, 0, R1).start(priority=BULK)

    def start_urgent(src_hbm, sg, c, j):
        slot_copy(src_hbm, sg, c, j, R1, RW - R1).start(priority=URGENT)

    def wait_slot(t):
        pltpu.make_async_copy(k_hbm.at[pl.ds(0, RW), pl.ds(0, CW)], ring.at[t], rsem.at[t]).wait()

    def wq_block(blk):
        c0 = pl.multiple_of(blk * QW, QW)
        return pltpu.make_async_copy(wq_hbm.at[:, pl.ds(c0, QW)], wq_v.at[blk], wqsem.at[blk])

    x_cp = pltpu.make_async_copy(x_hbm, x_v, msem.at[0])
    wr_cp = pltpu.make_async_copy(wr_hbm, wr_v, msem.at[1])
    wo_all = pltpu.make_async_copy(wo_hbm, wo_v, wosem.at[0])
    wg_all = pltpu.make_async_copy(wg_hbm, wg_v, wgsem.at[0])
    wu_all = pltpu.make_async_copy(wu_hbm, wu_v, wgsem.at[1])
    wd_cps = [pltpu.make_async_copy(wd_hbm.at[pl.ds(c * WDC, WDC)], wd_v.at[pl.ds(c * WDC, WDC)], wdsem.at[c])
              for c in range(NWD)]

    def start_weight_piece(e):
        @pl.when(e < E0)
        def _():
            ee = jnp.minimum(e, E0 - 1)
            blk = ee // NIT + 1
            i = ee % NIT
            r = pl.multiple_of((i // (QW // QC)) * QR, 8)
            cc = pl.multiple_of((i % (QW // QC)) * QC, QC)
            pltpu.make_async_copy(wq_hbm.at[pl.ds(r, QR), pl.ds(blk * QW + cc, QC)],
                                  wq_v.at[blk, pl.ds(r, QR), pl.ds(cc, QC)], wqsem.at[blk]).start(priority=URGENT)

        @pl.when(jnp.logical_and(e >= E0, e < E0 + NWOP))
        def _():
            r = pl.multiple_of(jnp.clip(e - E0, 0, NWOP - 1) * WOR, WOR)
            pltpu.make_async_copy(wo_hbm.at[pl.ds(r, WOR)], wo_v.at[pl.ds(r, WOR)],
                                  wosem.at[0]).start(priority=URGENT)

        for k, (w_hbm, w_v) in enumerate([(wg_hbm, wg_v), (wu_hbm, wu_v)]):
            lo = E0 + NWOP + k * NGP

            @pl.when(jnp.logical_and(e >= lo, e < lo + NGP))
            def _():
                i = jnp.clip(e - lo, 0, NGP - 1)
                cc = pl.multiple_of((i // NGR) * GC, GC)
                r = pl.multiple_of((i % NGR) * GR, 8)
                pltpu.make_async_copy(w_hbm.at[pl.ds(r, GR), pl.ds(cc, GC)],
                                      w_v.at[pl.ds(r, GR), pl.ds(cc, GC)], wgsem.at[k]).start(priority=URGENT)

    def start_w_down():
        for cp in wd_cps:
            cp.start(priority=BULK)

    x_cp.start()
    wq_block(0).start()
    for c in range(DP):
        for j in range(NP):
            start_bulk(k_hbm, 0, c, j)
    for c in range(DL):
        for j in range(NP):
            start_urgent(k_hbm, 0, c, j)
    wr_cp.start()

    o_s[...] = jnp.zeros_like(o_s)
    x_cp.wait()
    xn_s[...] = jnp.concatenate([_ln(x_v[...].astype(jnp.float32)), jnp.zeros((8 - B, D), jnp.float32)],
                                axis=0).astype(jnp.bfloat16)
    rowi = lax.broadcasted_iota(jnp.int32, (8, RW), 0)
    lanei = lax.broadcasted_iota(jnp.int32, (8, RW), 1)
    half = (lanei >= DH).astype(jnp.int32)
    diag = [rowi == (2 * j + half) for j in range(NP)]
    scale = DH ** -0.5

    def ahead(start, dist, c, j, cur_hbm, cur_sg, nxt_hbm, nxt_sg, has_next):
        cc = c + dist
        pl.when(cc < NC)(lambda: start(cur_hbm, cur_sg, jnp.minimum(cc, NC - 1), j))
        cond = cc >= NC if has_next is True else jnp.logical_and(has_next, cc >= NC)
        pl.when(cond)(lambda: start(nxt_hbm, nxt_sg, jnp.maximum(cc - NC, 0), j))

    def iteration(n, compute, carry, cur_hbm, cur_sg, nxt_hbm, nxt_sg, has_next, final_phase, piece, hooks=None):
        slots = [(n * CPI + ci, j) for ci in range(CPI) for j in range(NP)]
        ctx = (cur_hbm, cur_sg, nxt_hbm, nxt_sg, has_next)
        carry = compute(n, carry)
        ahead(start_urgent, DL, *slots[0], *ctx)
        for (c, j) in slots:
            ahead(start_bulk, DP, c, j, *ctx)
        more = None if final_phase is False else jnp.logical_not(jnp.logical_and(final_phase, n == NIT - 1))
        for u in range(U):
            wait = functools.partial(wait_slot, (n * U + U + u) % NS)
            if more is None:
                wait()
            else:
                pl.when(more)(wait)
            if u >= 1:
                ahead(start_urgent, DL, *slots[u], *ctx)
            if hooks is not None and u in hooks:
                hooks[u](carry)
        if piece is not None:
            start_weight_piece(piece)
        if final_phase is not False:
            pl.when(jnp.logical_and(final_phase, n == (NC - DP) // CPI - 1))(start_w_down)
        return carry

    for t in range(U):
        wait_slot(t)

    def supergroup(sg, carry):
        @pl.when(sg < NQB)
        def _():
            blk = jnp.minimum(sg, NQB - 1)
            wq_block(blk).wait()
            qq = jnp.dot(xn_s[...], wq_v[blk], preferred_element_type=jnp.float32)
            for j in range(NP):
                for b in range(B):
                    qb = jnp.broadcast_to(qq[b:b + 1, j * RW:(j + 1) * RW], (8, RW))
                    q_s[b * PPB + blk * NP + j] = jnp.where(diag[j], qb, 0.0).astype(jnp.bfloat16)

        qs = [q_s[sg * NP + j] for j in range(NP)]

        def k_compute(n, m):
            for ci in range(CPI):
                c = n * CPI + ci
                s = None
                for j in range(NP):
                    sp = jnp.dot(qs[j], ring[c * NP + j], preferred_element_type=jnp.float32)
                    s = sp if s is None else s + sp
                s_s[c] = s
                m = jnp.maximum(m, s)
            return m

        def k_iter(n, m, hooks=None):
            return iteration(n, k_compute, m, k_hbm, sg, v_hbm, sg, True, False, sg * NIT + n, hooks)

        box = {}

        def row_max(m):
            box["max"] = jnp.max(m, axis=1, keepdims=True)

        m = lax.fori_loop(0, NIT - 1, k_iter, jnp.full((8, CW), -jnp.inf, jnp.float32))
        k_iter(NIT - 1, m, {1: row_max})
        mx = box["max"]

        is_last = sg == NSG - 1

        @pl.when(is_last)
        def _():
            wo_all.wait()
            oc = jnp.concatenate([o_s[i] for i in range(PPB)], axis=1).astype(jnp.bfloat16)
            attn_s[...] = jnp.dot(oc, wo_v[...], preferred_element_type=jnp.float32)

        def v_compute(n, carry):
            l, acc = carry
            acc = list(acc)
            for ci in range(CPI):
                c = n * CPI + ci
                p = jnp.exp((s_s[c] - mx) * scale)
                l = l + p
                p = p.astype(jnp.bfloat16)
                for j in range(NP):
                    acc[j] = acc[j] + lax.dot_general(p, ring[c * NP + j], (((1,), (1,)), ((), ())),
                                                      preferred_element_type=jnp.float32)
            return l, tuple(acc)

        def v_iter(n, cr, hooks=None):
            return iteration(n, v_compute, cr, v_hbm, sg, k_hbm, jnp.minimum(sg + 1, NSG - 1),
                             jnp.logical_not(is_last), is_last, None, hooks)

        b = (sg * NP) // PPB

        def denominator(cr):
            box["inv"] = 1.0 / jnp.sum(cr[0], axis=1, keepdims=True)

        def emit_pair(j, cr):
            on = jnp.where(diag[j], cr[1][j] * box["inv"], 0.0)
            orow = jnp.sum(on, axis=0, keepdims=True)
            hp = (sg * NP + j) % PPB
            o_s[hp] = jnp.where(rowi == b, jnp.broadcast_to(orow, (8, RW)), o_s[hp])

        init = (jnp.zeros((8, CW), jnp.float32), tuple(jnp.zeros((8, RW), jnp.float32) for _ in range(NP)))
        cr = lax.fori_loop(0, NIT - 1, v_iter, init)
        v_iter(NIT - 1, cr, {1: denominator, 2: functools.partial(emit_pair, 0), 3: functools.partial(emit_pair, 1)})
        return carry

    lax.fori_loop(0, NSG, supergroup, 0)

    last = [jnp.where(rowi == B - 1, o_s[PPB - NP + j], 0.0) for j in range(NP)]
    oc = jnp.concatenate(last, axis=1).astype(jnp.bfloat16)
    attn = attn_s[...] + jnp.dot(oc, wo_v[(PPB - NP) * RW:, :], preferred_element_type=jnp.float32)
    x8 = jnp.concatenate([x_v[...].astype(jnp.float32), jnp.zeros((8 - B, D), jnp.float32)], axis=0)
    hh = x8 + attn
    hn = _ln(hh)
    wr_cp.wait()
    wr = wr_v[...].astype(jnp.float32).reshape(1, D)
    gate = jax.nn.sigmoid(jnp.sum(hn * wr, axis=-1, keepdims=True))
    hb = hn.astype(jnp.bfloat16)
    wg_all.wait()
    wu_all.wait()
    gg = jnp.dot(hb, wg_v[...], preferred_element_type=jnp.float32)
    uu = jnp.dot(hb, wu_v[...], preferred_element_type=jnp.float32)
    act = (gg * jax.nn.sigmoid(gg) * uu).astype(jnp.bfloat16)
    y = jnp.zeros((8, D), jnp.float32)
    for c in range(NWD):
        wd_cps[c].wait()
        y = y + jnp.dot(act[:, c * WDC:(c + 1) * WDC], wd_v[c * WDC:(c + 1) * WDC, :],
                        preferred_element_type=jnp.float32)
    res = hh + hn + y * gate
    o_ref[...] = res[0:B].astype(o_ref.dtype)


@jax.jit
def pallas_sequential_preLN__mha_block_cached__moe_arch_mod__decode_kernel(
    A_x: jax.Array,
    A_k_cache: jax.Array,
    A_v_cache: jax.Array,
    A_wq: jax.Array,
    A_wo: jax.Array,
    B_x: jax.Array,
    B_w_r: jax.Array,
    B_w_gate: jax.Array,
    B_w_up: jax.Array,
    B_w_down: jax.Array,
):
    kt = jnp.swapaxes(A_k_cache, 2, 3).reshape(BH * DH, SK)
    vt = jnp.swapaxes(A_v_cache, 2, 3).reshape(BH * DH, SK)
    x = A_x.reshape(B, D)
    out = pl.pallas_call(
        _kernel,
        out_shape=jax.ShapeDtypeStruct((B, D), jnp.bfloat16),
        in_specs=[pl.BlockSpec(memory_space=pl.ANY)] * 9,
        out_specs=pl.BlockSpec(memory_space=pltpu.VMEM),
        scratch_shapes=[
            pltpu.VMEM((NS, RW, CW), jnp.bfloat16),
            pltpu.VMEM((NQB, D, QW), jnp.bfloat16),
            pltpu.VMEM((H * DH, D), jnp.bfloat16),
            pltpu.VMEM((D, F), jnp.bfloat16),
            pltpu.VMEM((D, F), jnp.bfloat16),
            pltpu.VMEM((F, D), jnp.bfloat16),
            pltpu.VMEM((B, D), jnp.bfloat16),
            pltpu.VMEM((D,), jnp.bfloat16),
            pltpu.VMEM((8, D), jnp.bfloat16),
            pltpu.VMEM((NPAIR, 8, RW), jnp.bfloat16),
            pltpu.VMEM((PPB, 8, RW), jnp.float32),
            pltpu.VMEM((NC, 8, CW), jnp.float32),
            pltpu.VMEM((8, D), jnp.float32),
            pltpu.SemaphoreType.DMA((NS,)),
            pltpu.SemaphoreType.DMA((NQB,)),
            pltpu.SemaphoreType.DMA((1,)),
            pltpu.SemaphoreType.DMA((2,)),
            pltpu.SemaphoreType.DMA((NWD,)),
            pltpu.SemaphoreType.DMA((2,)),
        ],
        compiler_params=pltpu.CompilerParams(
            vmem_limit_bytes=100 * 1024 * 1024,
            disable_bounds_checks=True,
            disable_semaphore_checks=True,
        ),
    )(x, kt, vt, A_wq, A_wo, B_w_r, B_w_gate, B_w_up, B_w_down)
    return out.reshape(B, 1, D)
```

```python
import functools
import jax
import jax.numpy as jnp
from jax import lax
from jax.experimental import pallas as pl
from jax.experimental.pallas import tpu as pltpu

B, D, H, SK, DH, F = 4, 640, 32, 8192, 192, 1536
BH = B * H
EPS = 1e-5

M = 4
GR8 = 8 * M
NGRP = BH * DH // GR8
GPH = DH // GR8
NH = 8
SGG = NH * GPH
RW = SGG * 8
LPH = GPH * 8
CW = 128
NC = SK // CW
NSG = BH // NH
HB = H // NH
QW = NH * DH
NSL = M * NC
U = 4
NIT = NSL // U
IPS = NC // U
BULK, URGENT = 1, 0


def _ln(x):
    m = jnp.mean(x, axis=-1, keepdims=True)
    xc = x - m
    v = jnp.mean(xc * xc, axis=-1, keepdims=True)
    return xc / jnp.sqrt(v + EPS)


def _make_kernel(N1=41, DP=24, DL=12, NWD=6, notail=False, do_compute=True):
    WDC = F // NWD
    QR, QC = 40, 384
    NQP = (D // QR) * (QW // QC)
    assert NQP == NIT
    WOG = 2
    NWOP = (H * GPH // WOG) * M
    GR, GC = 40, 256
    NGR = D // GR
    NGP = NGR * (F // GC)
    E0 = (HB - 1) * NIT
    assert E0 + NWOP + 2 * NGP <= (NSG - 2) * NIT
    PPAD = 8 * (M - 1)

    def kernel(x_hbm, k_hbm, v_hbm, wq_hbm, wo_hbm, wr_hbm, wg_hbm, wu_hbm, wd_hbm, o_ref,
               ring, wq_v, wo_v, wg_v, wu_v, wd_v, x_v, wr_v, xn_s, sel_s, q_s, o_s, s_s, p_s, attn_s,
               rsem, wqsem, wosem, wgsem, wdsem, msem):
        def slot_copy(src_hbm, sg, u, lo, n):
            s = u // NC
            c = u % NC
            c0 = pl.multiple_of(c * CW, CW)
            return pltpu.make_async_copy(src_hbm.at[pl.ds(sg * SGG + lo, n), s, :, pl.ds(c0, CW)],
                                         ring.at[c, pl.ds(lo, n)], rsem.at[c])

        def start_bulk(src_hbm, sg, u):
            slot_copy(src_hbm, sg, u, 0, N1).start(priority=BULK)

        def start_urgent(src_hbm, sg, u):
            slot_copy(src_hbm, sg, u, N1, SGG - N1).start(priority=URGENT)

        def wait_slot(c):
            pltpu.make_async_copy(k_hbm.at[pl.ds(0, SGG), 0, :, pl.ds(0, CW)], ring.at[c], rsem.at[c]).wait()

        def wq_block(blk):
            c0 = pl.multiple_of(blk * QW, QW)
            return pltpu.make_async_copy(wq_hbm.at[:, pl.ds(c0, QW)], wq_v.at[blk], wqsem.at[blk])

        x_cp = pltpu.make_async_copy(x_hbm, x_v, msem.at[0])
        wr_cp = pltpu.make_async_copy(wr_hbm, wr_v, msem.at[1])
        wo_all = pltpu.make_async_copy(wo_v, wo_v, wosem.at[0])
        wg_all = pltpu.make_async_copy(wg_hbm, wg_v, wgsem.at[0])
        wu_all = pltpu.make_async_copy(wu_hbm, wu_v, wgsem.at[1])
        wd_cps = [pltpu.make_async_copy(wd_hbm.at[pl.ds(c * WDC, WDC)], wd_v.at[pl.ds(c * WDC, WDC)], wdsem.at[c])
                  for c in range(NWD)]

        def start_weight_piece(e):
            @pl.when(e < E0)
            def _():
                ee = jnp.minimum(e, E0 - 1)
                blk = ee // NIT + 1
                i = ee % NIT
                r = pl.multiple_of((i // (QW // QC)) * QR, 8)
                cc = pl.multiple_of((i % (QW // QC)) * QC, QC)
                pltpu.make_async_copy(wq_hbm.at[pl.ds(r, QR), pl.ds(blk * QW + cc, QC)],
                                      wq_v.at[blk, pl.ds(r, QR), pl.ds(cc, QC)], wqsem.at[blk]).start(priority=URGENT)

            @pl.when(jnp.logical_and(e >= E0, e < E0 + NWOP))
            def _():
                i = jnp.clip(e - E0, 0, NWOP - 1)
                s = i % M
                g0 = (i // M) * WOG
                pltpu.make_async_copy(wo_hbm.at[pl.ds(g0, WOG), s], wo_v.at[s, pl.ds(g0, WOG)],
                                      wosem.at[0]).start(priority=URGENT)

            for k, (w_hbm, w_v) in enumerate([(wg_hbm, wg_v), (wu_hbm, wu_v)]):
                lo = E0 + NWOP + k * NGP

                @pl.when(jnp.logical_and(e >= lo, e < lo + NGP))
                def _():
                    i = jnp.clip(e - lo, 0, NGP - 1)
                    cc = pl.multiple_of((i // NGR) * GC, GC)
                    r = pl.multiple_of((i % NGR) * GR, 8)
                    pltpu.make_async_copy(w_hbm.at[pl.ds(r, GR), pl.ds(cc, GC)],
                                          w_v.at[pl.ds(r, GR), pl.ds(cc, GC)], wgsem.at[k]).start(priority=URGENT)

        def start_w_down():
            for cp in wd_cps:
                cp.start(priority=BULK)

        x_cp.start()
        wq_block(0).start()
        for u in range(DP):
            start_bulk(k_hbm, 0, u)
        for u in range(DL):
            start_urgent(k_hbm, 0, u)
        wr_cp.start()

        o_s[...] = jnp.zeros_like(o_s)
        s_s[...] = jnp.zeros_like(s_s)
        rr = lax.broadcasted_iota(jnp.int32, (QW + PPAD, RW), 0)
        ll = lax.broadcasted_iota(jnp.int32, (1, RW), 1)
        tgt = DH * (ll // LPH) + GR8 * ((ll % LPH) // 8) + ll % 8 + PPAD
        sel_s[...] = jnp.where(rr == tgt, 1.0, 0.0).astype(jnp.bfloat16)
        x_cp.wait()
        xn_s[...] = jnp.concatenate([_ln(x_v[...].astype(jnp.float32)), jnp.zeros((8 - B, D), jnp.float32)],
                                    axis=0).astype(jnp.bfloat16)
        rowi = lax.broadcasted_iota(jnp.int32, (8, RW), 0)
        lanei = lax.broadcasted_iota(jnp.int32, (8, RW), 1)
        diag = rowi == lanei // LPH
        scale = DH ** -0.5

        def ahead(start, dist, u, cur_hbm, cur_sg, nxt_hbm, nxt_sg, has_next):
            uu = u + dist
            pl.when(uu < NSL)(lambda: start(cur_hbm, cur_sg, jnp.minimum(uu, NSL - 1)))
            cond = uu >= NSL if has_next is True else jnp.logical_and(has_next, uu >= NSL)
            pl.when(cond)(lambda: start(nxt_hbm, nxt_sg, jnp.maximum(uu - NSL, 0)))

        def iteration(n, compute, carry, cur_hbm, cur_sg, nxt_hbm, nxt_sg, has_next, final_phase, piece, hooks=None):
            us = [n * U + i for i in range(U)]
            ctx = (cur_hbm, cur_sg, nxt_hbm, nxt_sg, has_next)
            carry = compute(n, carry)
            ahead(start_urgent, DL, us[0], *ctx)
            for u in us:
                ahead(start_bulk, DP, u, *ctx)
            more = None if final_phase is False else jnp.logical_not(jnp.logical_and(final_phase, n == NIT - 1))
            for i in range(U):
                wait = functools.partial(wait_slot, (n * U + U + i) % NC)
                if more is None:
                    wait()
                else:
                    pl.when(more)(wait)
                if i >= 1:
                    ahead(start_urgent, DL, us[i], *ctx)
                if hooks is not None and i in hooks:
                    carry = hooks[i](carry)
            if piece is not None:
                start_weight_piece(piece)
            if final_phase is not False:
                pl.when(jnp.logical_and(final_phase, n == (NSL - DP) // U - 1))(start_w_down)
            return carry

        for c in range(U):
            wait_slot(c)

        def supergroup(sg, carry):
            @pl.when(sg < HB)
            def _():
                blk = jnp.minimum(sg, HB - 1)
                wq_block(blk).wait()
                qq = jnp.dot(xn_s[...], wq_v[blk], preferred_element_type=jnp.float32).astype(jnp.bfloat16)
                for s in range(M):
                    lo = PPAD - 8 * s
                    y = jnp.dot(qq, sel_s[lo:lo + QW, :], preferred_element_type=jnp.float32)
                    for b in range(B):
                        qb = jnp.broadcast_to(y[b:b + 1], (8, RW))
                        q_s[(b * HB + blk) * M + s] = jnp.where(diag, qb, 0.0).astype(jnp.bfloat16)

            def k_compute(n, carry):
                if not do_compute:
                    return carry
                s = n // IPS
                lhs = q_s[sg * M + s]
                for i in range(U):
                    c = (n * U + i) % NC
                    sp = jnp.dot(lhs, ring[c].reshape(RW, CW), preferred_element_type=jnp.float32)
                    s_s[c] = jnp.where(s == 0, sp, s_s[c] + sp)
                return carry

            def k_iter(n, carry, hooks=None):
                return iteration(n, k_compute, carry, k_hbm, sg, v_hbm, sg, True, False, sg * NIT + n, hooks)

            box = {}

            def row_max(carry):
                m = s_s[0]
                for c in range(1, NC):
                    m = jnp.maximum(m, s_s[c])
                box["max"] = jnp.max(m, axis=1, keepdims=True)
                return carry

            def probs(lo, hi, carry):
                l = box.get("l")
                for c in range(lo, hi):
                    p = jnp.exp((s_s[c] - box["max"]) * scale)
                    l = p if l is None else l + p
                    p_s[c] = p.astype(jnp.bfloat16)
                box["l"] = l
                if hi == NC:
                    box["inv"] = 1.0 / jnp.sum(l, axis=1, keepdims=True)
                return carry

            lax.fori_loop(0, NIT - 1, k_iter, 0)
            k_iter(NIT - 1, 0, {1: row_max, 2: functools.partial(probs, 0, NC // 2), 3: functools.partial(probs, NC // 2, NC)})
            inv = box["inv"]

            is_last = sg == NSG - 1

            @pl.when(is_last)
            def _():
                wo_all.wait()
                acc = None
                for s in range(M):
                    oc = jnp.concatenate([o_s[s * HB + hb] for hb in range(HB)], axis=1).astype(jnp.bfloat16)
                    d = jnp.dot(oc, wo_v[s].reshape(QW, D), preferred_element_type=jnp.float32)
                    acc = d if acc is None else acc + d
                attn_s[...] = acc

            def v_compute(n, acc):
                if not do_compute:
                    return acc
                for i in range(U):
                    c = (n * U + i) % NC
                    acc = acc + lax.dot_general(p_s[c], ring[c].reshape(RW, CW), (((1,), (1,)), ((), ())),
                                                preferred_element_type=jnp.float32)
                return acc

            def v_iter(n, acc, hooks=None):
                return iteration(n, v_compute, acc, v_hbm, sg, k_hbm, jnp.minimum(sg + 1, NSG - 1),
                                 jnp.logical_not(is_last), is_last, None, hooks)

            b = sg // HB
            hb = sg % HB

            def sweep(s, carry):
                def emit(acc):
                    on = jnp.where(diag, acc * inv, 0.0)
                    orow = jnp.sum(on, axis=0, keepdims=True)
                    idx = s * HB + hb
                    o_s[idx] = jnp.where(rowi == b, jnp.broadcast_to(orow, (8, RW)), o_s[idx])
                    return acc
                acc = lax.fori_loop(s * IPS, s * IPS + IPS - 1, v_iter, jnp.zeros((8, RW), jnp.float32))
                v_iter(s * IPS + IPS - 1, acc, {1: emit})
                return carry

            lax.fori_loop(0, M, sweep, 0)
            return carry

        lax.fori_loop(0, NSG, supergroup, 0)

        x4 = x_v[...].astype(jnp.float32)
        if notail:
            wr_cp.wait(); wg_all.wait(); wu_all.wait()
            for c in range(NWD):
                wd_cps[c].wait()
            o_ref[...] = x4.astype(o_ref.dtype)
            return
        attn = attn_s[...]
        for s in range(M):
            oc = jnp.where(rowi == B - 1, o_s[s * HB + HB - 1], 0.0).astype(jnp.bfloat16)
            attn = attn + jnp.dot(oc, wo_v[s, (HB - 1) * SGG:, :, :].reshape(RW, D), preferred_element_type=jnp.float32)
        x8 = jnp.concatenate([x4, jnp.zeros((8 - B, D), jnp.float32)], axis=0)
        hh = x8 + attn
        hn = _ln(hh)
        wr_cp.wait()
        wr = wr_v[...].astype(jnp.float32).reshape(1, D)
        gate = jax.nn.sigmoid(jnp.sum(hn * wr, axis=-1, keepdims=True))
        hb16 = hn.astype(jnp.bfloat16)
        wg_all.wait()
        wu_all.wait()
        gg = jnp.dot(hb16, wg_v[...], preferred_element_type=jnp.float32)
        uu = jnp.dot(hb16, wu_v[...], preferred_element_type=jnp.float32)
        act = (gg * jax.nn.sigmoid(gg) * uu).astype(jnp.bfloat16)
        y = jnp.zeros((8, D), jnp.float32)
        for c in range(NWD):
            wd_cps[c].wait()
            y = y + jnp.dot(act[:, c * WDC:(c + 1) * WDC], wd_v[c * WDC:(c + 1) * WDC, :],
                            preferred_element_type=jnp.float32)
        res = hh + hn + y * gate
        o_ref[...] = res[0:B].astype(o_ref.dtype)

    @jax.jit
    def f(A_x, A_k_cache, A_v_cache, A_wq, A_wo, B_x, B_w_r, B_w_gate, B_w_up, B_w_down):
        kt = jnp.swapaxes(A_k_cache, 2, 3).reshape(NGRP, M, 8, SK)
        vt = jnp.swapaxes(A_v_cache, 2, 3).reshape(NGRP, M, 8, SK)
        wo4 = A_wo.reshape(H * GPH, M, 8, D)
        x = A_x.reshape(B, D)
        out = pl.pallas_call(
            kernel,
            out_shape=jax.ShapeDtypeStruct((B, D), jnp.bfloat16),
            in_specs=[pl.BlockSpec(memory_space=pl.ANY)] * 9,
            out_specs=pl.BlockSpec(memory_space=pltpu.VMEM),
            scratch_shapes=[
                pltpu.VMEM((NC, SGG, 8, CW), jnp.bfloat16),
                pltpu.VMEM((HB, D, QW), jnp.bfloat16),
                pltpu.VMEM((M, H * GPH, 8, D), jnp.bfloat16),
                pltpu.VMEM((D, F), jnp.bfloat16),
                pltpu.VMEM((D, F), jnp.bfloat16),
                pltpu.VMEM((F, D), jnp.bfloat16),
                pltpu.VMEM((B, D), jnp.bfloat16),
                pltpu.VMEM((D,), jnp.bfloat16),
                pltpu.VMEM((8, D), jnp.bfloat16),
                pltpu.VMEM((QW + PPAD, RW), jnp.bfloat16),
                pltpu.VMEM((NSG * M, 8, RW), jnp.bfloat16),
                pltpu.VMEM((M * HB, 8, RW), jnp.float32),
                pltpu.VMEM((NC, 8, CW), jnp.float32),
                pltpu.VMEM((NC, 8, CW), jnp.bfloat16),
                pltpu.VMEM((8, D), jnp.float32),
                pltpu.SemaphoreType.DMA((NC,)),
                pltpu.SemaphoreType.DMA((HB,)),
                pltpu.SemaphoreType.DMA((1,)),
                pltpu.SemaphoreType.DMA((2,)),
                pltpu.SemaphoreType.DMA((NWD,)),
                pltpu.SemaphoreType.DMA((2,)),
            ],
            compiler_params=pltpu.CompilerParams(vmem_limit_bytes=100 * 1024 * 1024, disable_bounds_checks=True,
                                                 disable_semaphore_checks=True),
        )(x, kt, vt, A_wq, wo4, B_w_r, B_w_gate, B_w_up, B_w_down)
        return out.reshape(B, 1, D)

    return f


_impl = _make_kernel()


@jax.jit
def pallas_sequential_preLN__mha_block_cached__moe_arch_mod__decode_kernel(
    A_x, A_k_cache, A_v_cache, A_wq, A_wo, B_x, B_w_r, B_w_gate, B_w_up, B_w_down):
    return _impl(A_x, A_k_cache, A_v_cache, A_wq, A_wo, B_x, B_w_r, B_w_gate, B_w_up, B_w_down)
```

```python
import functools

import jax
import jax.numpy as jnp
from jax import lax
from jax.experimental import pallas as pl
from jax.experimental.pallas import tpu as pltpu

B, D, H, SK, DH, F = 4, 640, 32, 8192, 192, 1536
BH = B * H
EPS = 1e-5

M = 4
GR8 = 8 * M
NGRP = BH * DH // GR8
GPH = DH // GR8
NH = 8
SGG = NH * GPH
RW = SGG * 8
LPH = GPH * 8
CW = 128
NC = SK // CW
NSG = BH // NH
HB = H // NH
QW = NH * DH
NSL = M * NC
U = 4
NIT = NSL // U
IPS = NC // U

N1 = 41
DP = 24
DL = 12
BULK, URGENT = 1, 0

QR, QC = 40, 384
WOG = 2
NWOP = (H * GPH // WOG) * M
GR, GC = 40, 256
NGR = D // GR
NGP = NGR * (F // GC)
E0 = (HB - 1) * NIT
NWD = 6
WDC = F // NWD
PPAD = 8 * (M - 1)
assert (D // QR) * (QW // QC) == NIT
assert E0 + NWOP + 2 * NGP <= (NSG - 2) * NIT


def _ln(x):
    m = jnp.mean(x, axis=-1, keepdims=True)
    xc = x - m
    v = jnp.mean(xc * xc, axis=-1, keepdims=True)
    return xc / jnp.sqrt(v + EPS)


def _kernel(x_hbm, k_hbm, v_hbm, wq_hbm, wo_hbm, wr_hbm, wg_hbm, wu_hbm, wd_hbm, o_ref,
            ring, wq_v, wo_v, wg_v, wu_v, wd_v, x_v, wr_v, xn_s, sel_s, q_s, o_s, s_s, p_s, attn_s,
            rsem, wqsem, wosem, wgsem, wdsem, msem):
    def slot_copy(src_hbm, sg, u, lo, n):
        s = u // NC
        c = u % NC
        c0 = pl.multiple_of(c * CW, CW)
        return pltpu.make_async_copy(src_hbm.at[pl.ds(sg * SGG + lo, n), s, :, pl.ds(c0, CW)],
                                     ring.at[c, pl.ds(lo, n)], rsem.at[c])

    def start_bulk(src_hbm, sg, u):
        slot_copy(src_hbm, sg, u, 0, N1).start(priority=BULK)

    def start_urgent(src_hbm, sg, u):
        slot_copy(src_hbm, sg, u, N1, SGG - N1).start(priority=URGENT)

    def wait_slot(c):
        pltpu.make_async_copy(k_hbm.at[pl.ds(0, SGG), 0, :, pl.ds(0, CW)], ring.at[c], rsem.at[c]).wait()

    def wq_block(blk):
        c0 = pl.multiple_of(blk * QW, QW)
        return pltpu.make_async_copy(wq_hbm.at[:, pl.ds(c0, QW)], wq_v.at[blk], wqsem.at[blk])

    x_cp = pltpu.make_async_copy(x_hbm, x_v, msem.at[0])
    wr_cp = pltpu.make_async_copy(wr_hbm, wr_v, msem.at[1])
    wo_all = pltpu.make_async_copy(wo_v, wo_v, wosem.at[0])
    wg_all = pltpu.make_async_copy(wg_hbm, wg_v, wgsem.at[0])
    wu_all = pltpu.make_async_copy(wu_hbm, wu_v, wgsem.at[1])
    wd_cps = [pltpu.make_async_copy(wd_hbm.at[pl.ds(c * WDC, WDC)], wd_v.at[pl.ds(c * WDC, WDC)], wdsem.at[c])
              for c in range(NWD)]

    def start_weight_piece(e):
        @pl.when(e < E0)
        def _():
            ee = jnp.minimum(e, E0 - 1)
            blk = ee // NIT + 1
            i = ee % NIT
            r = pl.multiple_of((i // (QW // QC)) * QR, 8)
            cc = pl.multiple_of((i % (QW // QC)) * QC, QC)
            pltpu.make_async_copy(wq_hbm.at[pl.ds(r, QR), pl.ds(blk * QW + cc, QC)],
                                  wq_v.at[blk, pl.ds(r, QR), pl.ds(cc, QC)], wqsem.at[blk]).start(priority=URGENT)

        @pl.when(jnp.logical_and(e >= E0, e < E0 + NWOP))
        def _():
            i = jnp.clip(e - E0, 0, NWOP - 1)
            s = i % M
            g0 = (i // M) * WOG
            pltpu.make_async_copy(wo_hbm.at[pl.ds(g0, WOG), s], wo_v.at[s, pl.ds(g0, WOG)],
                                  wosem.at[0]).start(priority=URGENT)

        for k, (w_hbm, w_v) in enumerate([(wg_hbm, wg_v), (wu_hbm, wu_v)]):
            lo = E0 + NWOP + k * NGP

            @pl.when(jnp.logical_and(e >= lo, e < lo + NGP))
            def _():
                i = jnp.clip(e - lo, 0, NGP - 1)
                cc = pl.multiple_of((i // NGR) * GC, GC)
                r = pl.multiple_of((i % NGR) * GR, 8)
                pltpu.make_async_copy(w_hbm.at[pl.ds(r, GR), pl.ds(cc, GC)],
                                      w_v.at[pl.ds(r, GR), pl.ds(cc, GC)], wgsem.at[k]).start(priority=URGENT)

    def start_w_down():
        for cp in wd_cps:
            cp.start(priority=BULK)

    x_cp.start()
    wq_block(0).start()
    for u in range(DP):
        start_bulk(k_hbm, 0, u)
    for u in range(DL):
        start_urgent(k_hbm, 0, u)
    wr_cp.start()

    o_s[...] = jnp.zeros_like(o_s)
    s_s[...] = jnp.zeros_like(s_s)
    rr = lax.broadcasted_iota(jnp.int32, (QW + PPAD, RW), 0)
    ll = lax.broadcasted_iota(jnp.int32, (1, RW), 1)
    tgt = DH * (ll // LPH) + GR8 * ((ll % LPH) // 8) + ll % 8 + PPAD
    sel_s[...] = jnp.where(rr == tgt, 1.0, 0.0).astype(jnp.bfloat16)
    x_cp.wait()
    xn_s[...] = jnp.concatenate([_ln(x_v[...].astype(jnp.float32)), jnp.zeros((8 - B, D), jnp.float32)],
                                axis=0).astype(jnp.bfloat16)
    rowi = lax.broadcasted_iota(jnp.int32, (8, RW), 0)
    lanei = lax.broadcasted_iota(jnp.int32, (8, RW), 1)
    diag = rowi == lanei // LPH
    scale = DH ** -0.5

    def ahead(start, dist, u, cur_hbm, cur_sg, nxt_hbm, nxt_sg, has_next):
        uu = u + dist
        pl.when(uu < NSL)(lambda: start(cur_hbm, cur_sg, jnp.minimum(uu, NSL - 1)))
        cond = uu >= NSL if has_next is True else jnp.logical_and(has_next, uu >= NSL)
        pl.when(cond)(lambda: start(nxt_hbm, nxt_sg, jnp.maximum(uu - NSL, 0)))

    def iteration(n, compute, carry, cur_hbm, cur_sg, nxt_hbm, nxt_sg, has_next, final_phase, piece, hooks=None):
        us = [n * U + i for i in range(U)]
        ctx = (cur_hbm, cur_sg, nxt_hbm, nxt_sg, has_next)
        carry = compute(n, carry)
        ahead(start_urgent, DL, us[0], *ctx)
        for u in us:
            ahead(start_bulk, DP, u, *ctx)
        more = None if final_phase is False else jnp.logical_not(jnp.logical_and(final_phase, n == NIT - 1))
        for i in range(U):
            wait = functools.partial(wait_slot, (n * U + U + i) % NC)
            if more is None:
                wait()
            else:
                pl.when(more)(wait)
            if i >= 1:
                ahead(start_urgent, DL, us[i], *ctx)
            if hooks is not None and i in hooks:
                hooks[i](carry)
        if piece is not None:
            start_weight_piece(piece)
        if final_phase is not False:
            pl.when(jnp.logical_and(final_phase, n == (NSL - DP) // U - 1))(start_w_down)
        return carry

    for c in range(U):
        wait_slot(c)

    def supergroup(sg, carry):
        @pl.when(sg < HB)
        def _():
            blk = jnp.minimum(sg, HB - 1)
            wq_block(blk).wait()
            qq = jnp.dot(xn_s[...], wq_v[blk], preferred_element_type=jnp.float32).astype(jnp.bfloat16)
            for s in range(M):
                lo = PPAD - 8 * s
                y = jnp.dot(qq, sel_s[lo:lo + QW, :], preferred_element_type=jnp.float32)
                for b in range(B):
                    qb = jnp.broadcast_to(y[b:b + 1], (8, RW))
                    q_s[(b * HB + blk) * M + s] = jnp.where(diag, qb, 0.0).astype(jnp.bfloat16)

        def k_compute(n, carry):
            s = n // IPS
            lhs = q_s[sg * M + s]
            for i in range(U):
                c = (n * U + i) % NC
                sp = jnp.dot(lhs, ring[c].reshape(RW, CW), preferred_element_type=jnp.float32)
                s_s[c] = jnp.where(s == 0, sp, s_s[c] + sp)
            return carry

        def k_iter(n, carry, hooks=None):
            return iteration(n, k_compute, carry, k_hbm, sg, v_hbm, sg, True, False, sg * NIT + n, hooks)

        box = {}

        def row_max(_):
            m = s_s[0]
            for c in range(1, NC):
                m = jnp.maximum(m, s_s[c])
            box["max"] = jnp.max(m, axis=1, keepdims=True)

        def probs(lo, hi, _):
            l = box.get("l")
            for c in range(lo, hi):
                p = jnp.exp((s_s[c] - box["max"]) * scale)
                l = p if l is None else l + p
                p_s[c] = p.astype(jnp.bfloat16)
            box["l"] = l
            if hi == NC:
                box["inv"] = 1.0 / jnp.sum(l, axis=1, keepdims=True)

        lax.fori_loop(0, NIT - 1, k_iter, 0)
        k_iter(NIT - 1, 0, {1: row_max, 2: functools.partial(probs, 0, NC // 2),
                            3: functools.partial(probs, NC // 2, NC)})
        inv = box["inv"]

        is_last = sg == NSG - 1

        @pl.when(is_last)
        def _():
            wo_all.wait()
            acc = None
            for s in range(M):
                oc = jnp.concatenate([o_s[s * HB + hb] for hb in range(HB)], axis=1).astype(jnp.bfloat16)
                d = jnp.dot(oc, wo_v[s].reshape(HB * RW, D), preferred_element_type=jnp.float32)
                acc = d if acc is None else acc + d
            attn_s[...] = acc

        def v_compute(n, acc):
            for i in range(U):
                c = (n * U + i) % NC
                acc = acc + lax.dot_general(p_s[c], ring[c].reshape(RW, CW), (((1,), (1,)), ((), ())),
                                            preferred_element_type=jnp.float32)
            return acc

        def v_iter(n, acc, hooks=None):
            return iteration(n, v_compute, acc, v_hbm, sg, k_hbm, jnp.minimum(sg + 1, NSG - 1),
                             jnp.logical_not(is_last), is_last, None, hooks)

        b = sg // HB
        hb = sg % HB

        def sweep(s, carry):
            def emit(acc):
                on = jnp.where(diag, acc * inv, 0.0)
                orow = jnp.sum(on, axis=0, keepdims=True)
                idx = s * HB + hb
                o_s[idx] = jnp.where(rowi == b, jnp.broadcast_to(orow, (8, RW)), o_s[idx])

            acc = lax.fori_loop(s * IPS, s * IPS + IPS - 1, v_iter, jnp.zeros((8, RW), jnp.float32))
            v_iter(s * IPS + IPS - 1, acc, {1: emit})
            return carry

        lax.fori_loop(0, M, sweep, 0)
        return carry

    lax.fori_loop(0, NSG, supergroup, 0)

    attn = attn_s[...]
    for s in range(M):
        oc = jnp.where(rowi == B - 1, o_s[s * HB + HB - 1], 0.0).astype(jnp.bfloat16)
        attn = attn + jnp.dot(oc, wo_v[s, (HB - 1) * SGG:, :, :].reshape(RW, D), preferred_element_type=jnp.float32)
    x8 = jnp.concatenate([x_v[...].astype(jnp.float32), jnp.zeros((8 - B, D), jnp.float32)], axis=0)
    hh = x8 + attn
    hn = _ln(hh)
    wr_cp.wait()
    wr = wr_v[...].astype(jnp.float32).reshape(1, D)
    gate = jax.nn.sigmoid(jnp.sum(hn * wr, axis=-1, keepdims=True))
    hb16 = hn.astype(jnp.bfloat16)
    wg_all.wait()
    wu_all.wait()
    gg = jnp.dot(hb16, wg_v[...], preferred_element_type=jnp.float32)
    uu = jnp.dot(hb16, wu_v[...], preferred_element_type=jnp.float32)
    act = (gg * jax.nn.sigmoid(gg) * uu).astype(jnp.bfloat16)
    y = jnp.zeros((8, D), jnp.float32)
    for c in range(NWD):
        wd_cps[c].wait()
        y = y + jnp.dot(act[:, c * WDC:(c + 1) * WDC], wd_v[c * WDC:(c + 1) * WDC, :],
                        preferred_element_type=jnp.float32)
    res = hh + hn + y * gate
    o_ref[...] = res[0:B].astype(o_ref.dtype)


@jax.jit
def pallas_sequential_preLN__mha_block_cached__moe_arch_mod__decode_kernel(
    A_x: jax.Array,
    A_k_cache: jax.Array,
    A_v_cache: jax.Array,
    A_wq: jax.Array,
    A_wo: jax.Array,
    B_x: jax.Array,
    B_w_r: jax.Array,
    B_w_gate: jax.Array,
    B_w_up: jax.Array,
    B_w_down: jax.Array,
):
    kt = jnp.swapaxes(A_k_cache, 2, 3).reshape(NGRP, M, 8, SK)
    vt = jnp.swapaxes(A_v_cache, 2, 3).reshape(NGRP, M, 8, SK)
    wo4 = A_wo.reshape(H * GPH, M, 8, D)
    x = A_x.reshape(B, D)
    out = pl.pallas_call(
        _kernel,
        out_shape=jax.ShapeDtypeStruct((B, D), jnp.bfloat16),
        in_specs=[pl.BlockSpec(memory_space=pl.ANY)] * 9,
        out_specs=pl.BlockSpec(memory_space=pltpu.VMEM),
        scratch_shapes=[
            pltpu.VMEM((NC, SGG, 8, CW), jnp.bfloat16),
            pltpu.VMEM((HB, D, QW), jnp.bfloat16),
            pltpu.VMEM((M, H * GPH, 8, D), jnp.bfloat16),
            pltpu.VMEM((D, F), jnp.bfloat16),
            pltpu.VMEM((D, F), jnp.bfloat16),
            pltpu.VMEM((F, D), jnp.bfloat16),
            pltpu.VMEM((B, D), jnp.bfloat16),
            pltpu.VMEM((D,), jnp.bfloat16),
            pltpu.VMEM((8, D), jnp.bfloat16),
            pltpu.VMEM((QW + PPAD, RW), jnp.bfloat16),
            pltpu.VMEM((NSG * M, 8, RW), jnp.bfloat16),
            pltpu.VMEM((M * HB, 8, RW), jnp.float32),
            pltpu.VMEM((NC, 8, CW), jnp.float32),
            pltpu.VMEM((NC, 8, CW), jnp.bfloat16),
            pltpu.VMEM((8, D), jnp.float32),
            pltpu.SemaphoreType.DMA((NC,)),
            pltpu.SemaphoreType.DMA((HB,)),
            pltpu.SemaphoreType.DMA((1,)),
            pltpu.SemaphoreType.DMA((2,)),
            pltpu.SemaphoreType.DMA((NWD,)),
            pltpu.SemaphoreType.DMA((2,)),
        ],
        compiler_params=pltpu.CompilerParams(
            vmem_limit_bytes=100 * 1024 * 1024,
            disable_bounds_checks=True,
            disable_semaphore_checks=True,
        ),
    )(x, kt, vt, A_wq, wo4, B_w_r, B_w_gate, B_w_up, B_w_down)
    return out.reshape(B, 1, D)
```

```python
import functools

import jax
import jax.numpy as jnp
from jax import lax
from jax.experimental import pallas as pl
from jax.experimental.pallas import tpu as pltpu

B, D, H, SK, DH, F = 4, 640, 32, 8192, 192, 1536
BH = B * H
EPS = 1e-5

M = 4
GR8 = 8 * M
NGRP = BH * DH // GR8
GPH = DH // GR8
NH = 16
GPS = NH * GPH
SGG = 32
TP = GPS // SGG
RW = SGG * 8
CW = 128
NC = SK // CW
NSG = BH // NH
HB = H // NH
QP = SGG * GR8
NQB = HB * TP
NSW = TP * M
NSL = NSW * NC
U = 4
NIT = NSL // U
IPS = NC // U

N1 = 28
DP = 32
DL = 16
BULK, URGENT = 1, 0

QR, QC = 40, 256
PPP = (D // QR) * (QP // QC)
WOG = 2
NWOP = (H * GPH // WOG) * M
GR, GC = 40, 256
NGR = D // GR
NGP = NGR * (F // GC)
E0 = (NQB - 1) * PPP
NWD = 6
WDC = F // NWD
PPAD = 8 * (M - 1)
assert (NC, M, U, IPS, PPP, QP // QC, NGR, HB) == (64, 4, 4, 16, 64, 4, 16, 2)
assert PPP == M * IPS
assert E0 + NWOP + 2 * NGP <= (NSG - 1) * NIT
assert max(DP, DL) <= NC and DP + U <= NC


def _ln(x):
    m = jnp.mean(x, axis=-1, keepdims=True)
    xc = x - m
    v = jnp.mean(xc * xc, axis=-1, keepdims=True)
    return xc / jnp.sqrt(v + EPS)


def _kernel(x_hbm, k_hbm, v_hbm, wq_hbm, wo_hbm, wr_hbm, wg_hbm, wu_hbm, wd_hbm, o_ref,
            ring, wq_v, wo_v, wg_v, wu_v, wd_v, x_v, wr_v, xn_s, sel_s, q_s, o_s, s_s, p_s, attn_s,
            rsem, wqsem, wosem, wgsem, wdsem, msem):
    def slot_copy(src_hbm, sg, u, lo, n):
        c = u & (NC - 1)
        s = (u >> 6) & (M - 1)
        t = u >> 8
        c0 = pl.multiple_of(c * CW, CW)
        return pltpu.make_async_copy(src_hbm.at[pl.ds(sg * GPS + t * SGG + lo, n), s, :, pl.ds(c0, CW)],
                                     ring.at[c, pl.ds(lo, n)], rsem.at[c])

    def start_bulk(src_hbm, sg, u):
        slot_copy(src_hbm, sg, u, 0, N1).start(priority=BULK)

    def start_urgent(src_hbm, sg, u):
        slot_copy(src_hbm, sg, u, N1, SGG - N1).start(priority=URGENT)

    def wait_slot(c):
        pltpu.make_async_copy(k_hbm.at[pl.ds(0, SGG), 0, :, pl.ds(0, CW)], ring.at[c], rsem.at[c]).wait()

    def wq_part(j):
        c0 = pl.multiple_of(j * QP, QP)
        return pltpu.make_async_copy(wq_hbm.at[:, pl.ds(c0, QP)], wq_v.at[j], wqsem.at[j])

    x_cp = pltpu.make_async_copy(x_hbm, x_v, msem.at[0])
    wr_cp = pltpu.make_async_copy(wr_hbm, wr_v, msem.at[1])
    wo_all = pltpu.make_async_copy(wo_v, wo_v, wosem.at[0])
    wg_all = pltpu.make_async_copy(wg_hbm, wg_v, wgsem.at[0])
    wu_all = pltpu.make_async_copy(wu_hbm, wu_v, wgsem.at[1])
    wd_cps = [pltpu.make_async_copy(wd_hbm.at[pl.ds(c * WDC, WDC)], wd_v.at[pl.ds(c * WDC, WDC)], wdsem.at[c])
              for c in range(NWD)]

    def start_weight_piece(e):
        @pl.when(e < E0)
        def _():
            ee = jnp.minimum(e, E0 - 1)
            j = (ee >> 6) + 1
            i = ee & (PPP - 1)
            r = pl.multiple_of((i >> 2) * QR, 8)
            cc = pl.multiple_of((i & 3) * QC, QC)
            pltpu.make_async_copy(wq_hbm.at[pl.ds(r, QR), pl.ds(j * QP + cc, QC)],
                                  wq_v.at[j, pl.ds(r, QR), pl.ds(cc, QC)], wqsem.at[j]).start(priority=URGENT)

        @pl.when(jnp.logical_and(e >= E0, e < E0 + NWOP))
        def _():
            i = jnp.clip(e - E0, 0, NWOP - 1)
            s = i & (M - 1)
            g0 = (i >> 2) * WOG
            pltpu.make_async_copy(wo_hbm.at[pl.ds(g0, WOG), s], wo_v.at[s, pl.ds(g0, WOG)],
                                  wosem.at[0]).start(priority=URGENT)

        for k, (w_hbm, w_v) in enumerate([(wg_hbm, wg_v), (wu_hbm, wu_v)]):
            lo = E0 + NWOP + k * NGP

            @pl.when(jnp.logical_and(e >= lo, e < lo + NGP))
            def _():
                i = jnp.clip(e - lo, 0, NGP - 1)
                cc = pl.multiple_of((i >> 4) * GC, GC)
                r = pl.multiple_of((i & (NGR - 1)) * GR, 8)
                pltpu.make_async_copy(w_hbm.at[pl.ds(r, GR), pl.ds(cc, GC)],
                                      w_v.at[pl.ds(r, GR), pl.ds(cc, GC)], wgsem.at[k]).start(priority=URGENT)

    def start_w_down():
        for cp in wd_cps:
            cp.start(priority=BULK)

    x_cp.start()
    wq_part(0).start()
    for u in range(DP):
        start_bulk(k_hbm, 0, u)
    for u in range(DL):
        start_urgent(k_hbm, 0, u)
    wr_cp.start()

    o_s[...] = jnp.zeros_like(o_s)
    s_s[...] = jnp.zeros_like(s_s)
    rr = lax.broadcasted_iota(jnp.int32, (QP + PPAD, RW), 0)
    ll = lax.broadcasted_iota(jnp.int32, (1, RW), 1)
    tgt = GR8 * (ll >> 3) + (ll & 7) + PPAD
    sel_s[...] = jnp.where(rr == tgt, 1.0, 0.0).astype(jnp.bfloat16)
    x_cp.wait()
    xn_s[...] = jnp.concatenate([_ln(x_v[...].astype(jnp.float32)), jnp.zeros((8 - B, D), jnp.float32)],
                                axis=0).astype(jnp.bfloat16)
    row16 = lax.broadcasted_iota(jnp.int32, (NH, RW), 0)
    grp16 = lax.broadcasted_iota(jnp.int32, (NH, RW), 1) >> 3
    row8 = lax.broadcasted_iota(jnp.int32, (8, RW), 0)
    scale = DH ** -0.5

    def diag(t):
        g = grp16 + t * SGG
        return jnp.logical_and(g >= row16 * GPH, g < row16 * GPH + GPH)

    def iteration(n, compute, carry, cur_hbm, cur_sg, nxt, piece, hooks=None):
        us = [n * U + i for i in range(U)]

        def ahead(start, dist, u):
            uu = u + dist
            if nxt is None:
                start(cur_hbm, cur_sg, uu)
            else:
                nxt_hbm, nxt_sg, has_next, _ = nxt
                pl.when(uu < NSL)(lambda: start(cur_hbm, cur_sg, jnp.minimum(uu, NSL - 1)))
                cond = uu >= NSL if has_next is True else jnp.logical_and(has_next, uu >= NSL)
                pl.when(cond)(lambda: start(nxt_hbm, nxt_sg, jnp.maximum(uu - NSL, 0)))

        carry = compute(n, carry)
        ahead(start_urgent, DL, us[0])
        for u in us:
            ahead(start_bulk, DP, u)
        final_phase = False if nxt is None else nxt[3]
        more = None if final_phase is False else jnp.logical_not(jnp.logical_and(final_phase, n == NIT - 1))
        for i in range(U):
            wait = functools.partial(wait_slot, (n * U + U + i) & (NC - 1))
            if more is None:
                wait()
            else:
                pl.when(more)(wait)
            if i >= 1:
                ahead(start_urgent, DL, us[i])
            if hooks is not None and i in hooks:
                hooks[i](carry)
        if piece is not None:
            start_weight_piece(piece)
        if final_phase is not False:
            pl.when(jnp.logical_and(final_phase, n == (NSL - 1 - DP) // U))(start_w_down)
        return carry

    for c in range(U):
        wait_slot(c)

    def supergroup(sg, carry):
        def k_compute(n, carry):
            w = n >> 4
            lhs = q_s[sg * NSW + w]
            for i in range(U):
                c = (n * U + i) & (NC - 1)
                sp = jnp.dot(lhs, ring[c].reshape(RW, CW), preferred_element_type=jnp.float32)
                s_s[c] = jnp.where(w == 0, sp, s_s[c] + sp)
            return carry

        def k_iter(nxt, n, carry, hooks=None):
            return iteration(n, k_compute, carry, k_hbm, sg, nxt, sg * NIT + n, hooks)

        def k_sweep(w, carry):
            @pl.when(jnp.logical_and(sg < HB, (w & (M - 1)) == 0))
            def _():
                t = w >> 2
                j = jnp.minimum(sg, HB - 1) * TP + t
                wq_part(j).wait()
                qq = jnp.dot(xn_s[...], wq_v[j], preferred_element_type=jnp.float32).astype(jnp.bfloat16)
                dg = diag(t)
                for s in range(M):
                    lo = PPAD - 8 * s
                    y = jnp.dot(qq, sel_s[lo:lo + QP, :], preferred_element_type=jnp.float32)
                    for b in range(B):
                        qb = jnp.broadcast_to(y[b:b + 1], (NH, RW))
                        q_s[(b * NQB + j) * M + s] = jnp.where(dg, qb, 0.0).astype(jnp.bfloat16)
            return lax.fori_loop(w * IPS, w * IPS + IPS, functools.partial(k_iter, None), carry)

        box = {}

        def row_max(_):
            m = s_s[0]
            for c in range(1, NC):
                m = jnp.maximum(m, s_s[c])
            box["max"] = jnp.max(m, axis=1, keepdims=True)

        def probs(lo, hi, _):
            l = box.get("l")
            for c in range(lo, hi):
                p = jnp.exp((s_s[c] - box["max"]) * scale)
                l = p if l is None else l + p
                p_s[c] = p.astype(jnp.bfloat16)
            box["l"] = l
            if hi == NC:
                box["inv"] = 1.0 / jnp.sum(l, axis=1, keepdims=True)

        lax.fori_loop(0, NSW - 1, k_sweep, 0)
        knxt = (v_hbm, sg, True, False)
        lax.fori_loop((NSW - 1) * IPS, NIT - 1, functools.partial(k_iter, knxt), 0)
        k_iter(knxt, NIT - 1, 0, {1: row_max, 2: functools.partial(probs, 0, NC // 2),
                                  3: functools.partial(probs, NC // 2, NC)})
        inv = box["inv"]

        is_last = sg == NSG - 1
        b = sg >> 1
        hb = sg & 1

        def v_compute(n, acc):
            for i in range(U):
                c = (n * U + i) & (NC - 1)
                acc = acc + lax.dot_general(p_s[c], ring[c].reshape(RW, CW), (((1,), (1,)), ((), ())),
                                            preferred_element_type=jnp.float32)
            return acc

        def v_iter(nxt, n, acc, hooks=None):
            return iteration(n, v_compute, acc, v_hbm, sg, nxt, None, hooks)

        def v_sweep(nxt, w, carry):
            def emit(acc):
                t = w >> 2
                s = w & (M - 1)
                on = jnp.where(diag(t), acc * inv, 0.0)
                orow = jnp.sum(on, axis=0, keepdims=True)
                idx = (s * HB + hb) * TP + t
                o_s[idx] = jnp.where(row8 == b, jnp.broadcast_to(orow, (8, RW)), o_s[idx])

            acc = lax.fori_loop(w * IPS, w * IPS + IPS - 1, functools.partial(v_iter, nxt),
                                jnp.zeros((NH, RW), jnp.float32))
            v_iter(nxt, w * IPS + IPS - 1, acc, {1: emit})
            return carry

        def v_sweep_main(w, carry):
            @pl.when(jnp.logical_and(is_last, w == NSW - M))
            def _():
                wo_all.wait()
                acc = None
                for s in range(M):
                    oc = jnp.concatenate([o_s[s * NQB + i] for i in range(NQB)], axis=1).astype(jnp.bfloat16)
                    d = jnp.dot(oc, wo_v[s].reshape(NQB * RW, D), preferred_element_type=jnp.float32)
                    acc = d if acc is None else acc + d
                attn_s[...] = acc
            return v_sweep(None, w, carry)

        lax.fori_loop(0, NSW - 1, v_sweep_main, 0)
        vnxt = (k_hbm, jnp.minimum(sg + 1, NSG - 1), jnp.logical_not(is_last), is_last)
        v_sweep(vnxt, NSW - 1, 0)
        return carry

    lax.fori_loop(0, NSG, supergroup, 0)

    attn = attn_s[...]
    for s in range(M):
        oc = jnp.where(row8 == B - 1, o_s[s * NQB + NQB - 1], 0.0).astype(jnp.bfloat16)
        attn = attn + jnp.dot(oc, wo_v[s, (NQB - 1) * SGG:, :, :].reshape(RW, D),
                              preferred_element_type=jnp.float32)
    x8 = jnp.concatenate([x_v[...].astype(jnp.float32), jnp.zeros((8 - B, D), jnp.float32)], axis=0)
    hh = x8 + attn
    hn = _ln(hh)
    wr_cp.wait()
    wr = wr_v[...].astype(jnp.float32).reshape(1, D)
    gate = jax.nn.sigmoid(jnp.sum(hn * wr, axis=-1, keepdims=True))
    hb16 = hn.astype(jnp.bfloat16)
    wg_all.wait()
    wu_all.wait()
    gg = jnp.dot(hb16, wg_v[...], preferred_element_type=jnp.float32)
    uu = jnp.dot(hb16, wu_v[...], preferred_element_type=jnp.float32)
    act = (gg * jax.nn.sigmoid(gg) * uu).astype(jnp.bfloat16)
    y = jnp.zeros((8, D), jnp.float32)
    for c in range(NWD):
        wd_cps[c].wait()
        y = y + jnp.dot(act[:, c * WDC:(c + 1) * WDC], wd_v[c * WDC:(c + 1) * WDC, :],
                        preferred_element_type=jnp.float32)
    res = hh + hn + y * gate
    o_ref[...] = res[0:B].astype(o_ref.dtype)


assert (NSW - 1) * NC - 1 + max(DP, DL) < NSL


@jax.jit
def pallas_sequential_preLN__mha_block_cached__moe_arch_mod__decode_kernel(
        A_x, A_k_cache, A_v_cache, A_wq, A_wo, B_x, B_w_r, B_w_gate, B_w_up, B_w_down):
    del B_x
    kt = jnp.swapaxes(A_k_cache, 2, 3).reshape(NGRP, M, 8, SK)
    vt = jnp.swapaxes(A_v_cache, 2, 3).reshape(NGRP, M, 8, SK)
    wo4 = A_wo.reshape(H * GPH, M, 8, D)
    x = A_x.reshape(B, D)
    out = pl.pallas_call(
        _kernel,
        out_shape=jax.ShapeDtypeStruct((B, D), jnp.bfloat16),
        in_specs=[pl.BlockSpec(memory_space=pl.ANY)] * 9,
        out_specs=pl.BlockSpec(memory_space=pltpu.VMEM),
        scratch_shapes=[
            pltpu.VMEM((NC, SGG, 8, CW), jnp.bfloat16),
            pltpu.VMEM((NQB, D, QP), jnp.bfloat16),
            pltpu.VMEM((M, H * GPH, 8, D), jnp.bfloat16),
            pltpu.VMEM((D, F), jnp.bfloat16),
            pltpu.VMEM((D, F), jnp.bfloat16),
            pltpu.VMEM((F, D), jnp.bfloat16),
            pltpu.VMEM((B, D), jnp.bfloat16),
            pltpu.VMEM((D,), jnp.bfloat16),
            pltpu.VMEM((8, D), jnp.bfloat16),
            pltpu.VMEM((QP + PPAD, RW), jnp.bfloat16),
            pltpu.VMEM((NSG * NSW, NH, RW), jnp.bfloat16),
            pltpu.VMEM((M * NQB, 8, RW), jnp.float32),
            pltpu.VMEM((NC, NH, CW), jnp.float32),
            pltpu.VMEM((NC, NH, CW), jnp.bfloat16),
            pltpu.VMEM((8, D), jnp.float32),
            pltpu.SemaphoreType.DMA((NC,)),
            pltpu.SemaphoreType.DMA((NQB,)),
            pltpu.SemaphoreType.DMA((1,)),
            pltpu.SemaphoreType.DMA((2,)),
            pltpu.SemaphoreType.DMA((NWD,)),
            pltpu.SemaphoreType.DMA((2,)),
        ],
        compiler_params=pltpu.CompilerParams(vmem_limit_bytes=100 * 1024 * 1024, disable_bounds_checks=True,
                                             disable_semaphore_checks=True),
    )(x, kt, vt, A_wq, wo4, B_w_r, B_w_gate, B_w_up, B_w_down)
    return out.reshape(B, 1, D)
```
